```python
import jax
import jax.numpy as jnp

def _softmax(x, axis=-1):
    return jax.nn.softmax(x, axis=axis)
def _gelu(x):
    return jax.nn.gelu(x, approximate=True)
def _silu(x):
    return jax.nn.silu(x)
def _sigmoid(x):
    return jax.nn.sigmoid(x)
def _layernorm(x, axis=-1, eps=1e-5):
    m = jnp.mean(x, axis=axis, keepdims=True)
    v = jnp.var(x, axis=axis, keepdims=True)
    return (x - m) / jnp.sqrt(v + eps)
def _scatter_add(tgt, idx, src, axis=0):
    return tgt.at[idx].add(src)
def _segment_sum(src, seg, n):
    return jax.ops.segment_sum(src, seg, n)
class _Rng:
    def __init__(self, key):
        self._k = key
    def _next(self):
        self._k, sub = jax.random.split(self._k)
        return sub
    def normal(self, shape):
        return jax.random.normal(self._next(), shape, dtype=jnp.bfloat16)
    def randint(self, lo, hi, shape):
        return jax.random.randint(self._next(), shape, lo, hi, dtype=jnp.int32)
    def uniform(self, shape, lo=0.0, hi=1.0):
        return jax.random.uniform(self._next(), shape, jnp.bfloat16, lo, hi)
    def permutation(self, n):
        return jax.random.permutation(self._next(), n)


kernel_name = 'interleave_layers__sliding_local_dilated__glu_gated_geglu__prompt'

def setup_inputs():
    _rng = _Rng(jax.random.key(int.from_bytes(__import__("os").urandom(4), "little")))
    _w = (lambda a: (lambda t: t.astype(jnp.bfloat16) if jnp.issubdtype(t.dtype, jnp.floating) else t)(jnp.asarray(a)))
    def _A_setup():
        B, S, D = 1, 2048, 576
        return {
            "x": _w((lambda *s: _rng.normal(s) * 0.05)(B, S, D)),
            "wqkv": _w((lambda *s: _rng.normal(s) * 0.05)(D, 3 * D)),
            "wo": _w((lambda *s: _rng.normal(s) * 0.05)(D, D)),
        }
    _A_in = _A_setup()

    def _B_setup():
        B, S, Dm, Df = 1, 2048, 576, 4608
        return {
            "x": _w((lambda *s: _rng.normal(s) * 0.05)(B, S, Dm)),
            "w_gate": _w((lambda *s: _rng.normal(s) * 0.05)(Dm, Df) * (Dm ** -0.5)),
            "w_up": _w((lambda *s: _rng.normal(s) * 0.05)(Dm, Df) * (Dm ** -0.5)),
            "w_down": _w((lambda *s: _rng.normal(s) * 0.05)(Df, Dm) * (Df ** -0.5)),
        }
    _B_in = _B_setup()

    return {
        "A_x": _A_in["x"],
        "A_wqkv": _A_in["wqkv"],
        "A_wo": _A_in["wo"],
        "B_x": _B_in["x"],
        "B_w_gate": _B_in["w_gate"],
        "B_w_up": _B_in["w_up"],
        "B_w_down": _B_in["w_down"],
    }

def reference(A_x, A_wqkv, A_wo, B_x, B_w_gate, B_w_up, B_w_down):
    def _A_ref(x, wqkv, wo):
        B, S, D = x.shape
        H = 32; Dh = D // H
        W, dil = 8, 2
        qkv = (lambda x, *d: x.transpose(*d))((x @ wqkv).reshape(B, S, 3, H, Dh), 2, 0, 3, 1, 4)
        q, k, v = qkv[0], qkv[1], qkv[2]
        scale = Dh ** -0.5
        pos = jnp.arange(S)
        off = jnp.arange(W) * dil
        idx = pos[:, None] - off[None, :]
        mask = idx >= 0
        idx_c = jnp.where(mask, idx, 0).reshape(-1)
        kg = k[:, :, idx_c, :].reshape(B, H, S, W, Dh)
        vg = v[:, :, idx_c, :].reshape(B, H, S, W, Dh)
        logits = jnp.einsum("bhsd,bhswd->bhsw", q, kg) * scale
        logits = jnp.where(mask[None, None, :, :], logits, -1e9)
        attn = _softmax(logits, axis=-1)
        o = jnp.einsum("bhsw,bhswd->bhsd", attn, vg)
        return (lambda x, *d: x.transpose(*d))(o, 0, 2, 1, 3).reshape(B, S, D) @ wo

    def _B_ref(x, w_gate, w_up, w_down):
        g = jnp.einsum("bsd,df->bsf", x, w_gate)
        u = jnp.einsum("bsd,df->bsf", x, w_up)
        h = _gelu(g) * u
        return jnp.einsum("bsf,fd->bsd", h, w_down)

    x = A_x
    x = x + _A_ref(_layernorm(x, axis=-1), A_wqkv, A_wo)
    x = x + _B_ref(_layernorm(x, axis=-1), B_w_gate, B_w_up, B_w_down)
    x = x + _A_ref(_layernorm(x, axis=-1), A_wqkv, A_wo)
    x = x + _B_ref(_layernorm(x, axis=-1), B_w_gate, B_w_up, B_w_down)
    return x
```

```python
import functools
import numpy as np
import jax
import jax.numpy as jnp
from jax import lax
import jax.experimental.pallas as pl
import jax.experimental.pallas.tpu as pltpu

S, D, DF, H, DH, W, DIL = 2048, 576, 4608, 32, 18, 8, 2
DP = 640
NP = 5
HALO = 16
LOG2E = 1.4426950408889634
QSCALE = float(DH ** -0.5) * LOG2E
F32, BF16 = jnp.float32, jnp.bfloat16
NT = (((1,), (1,)), ((), ()))
TN = (((0,), (0,)), ((), ()))


def _ln_T(xT):
    m = jnp.mean(xT, axis=0, keepdims=True)
    xc = xT - m
    v = jnp.mean(xc * xc, axis=0, keepdims=True)
    return xc * lax.rsqrt(v + 1e-5)


def _gelu_mul(g, u):
    c0 = 0.7978845608028654
    c1 = 0.7978845608028654 * 0.044715
    inner = g * (c0 + c1 * (g * g))
    t = jnp.tanh(inner)
    hg = 0.5 * g
    return (hg + hg * t) * u


def make(TM=512, FC=512, plan=None, ASL=None):
    NB = S // TM
    NC = DF // FC
    if ASL is None:
        ASL = 64
    NS = TM // ASL

    def kernel(x0_ref, x1_ref, wqkv_hbm, wo_hbm, wg_hbm, wu_hbm, wdT_hbm, out_ref,
               wqkv_v, wo_v, wqp, wopT, wg_v, wu_v, wd_v,
               xres, xnA, xnF, qbuf, kbuf, vbuf, obuf, sems):
        n = pl.program_id(0)
        bF = n & (NB - 1)
        sF = n & 1

        def a_ln(b):
            xnA[...] = _ln_T(xres[b]).astype(BF16).T

        def a_q():
            qv = jnp.dot(xnA[...], wqp[0], preferred_element_type=F32)
            for j in range(NP):
                qbuf[j] = qv[:, j * 128:(j + 1) * 128] * QSCALE

        def a_kv(b, c, buf):
            old = [buf[j, pl.ds(TM, HALO), :] for j in range(NP)]
            kv = jnp.dot(xnA[...], wqp[c], preferred_element_type=F32)
            for j in range(NP):
                kj = kv[:, j * 128:(j + 1) * 128]
                buf[j, pl.ds(HALO, TM), :] = kj
                buf[j, pl.ds(0, HALO), :] = jnp.where(b == 0, jnp.broadcast_to(kj[0:1, :], (HALO, 128)), old[j])

        def a_core16(b, r, masked):
            q = [qbuf[j, pl.ds(r, 16), :] for j in range(NP)]
            lg = []
            for w in range(W):
                o = HALO - DIL * w
                acc = q[0] * kbuf[0, pl.ds(r + o, 16), :]
                for j in range(1, NP):
                    acc = acc + q[j] * kbuf[j, pl.ds(r + o, 16), :]
                acc = acc + pltpu.roll(acc, 64, 1)
                acc = acc + pltpu.roll(acc, 32, 1)
                if masked and w > 0:
                    row = lax.broadcasted_iota(jnp.int32, (16, 128), 0) + (b * TM + r - DIL * w)
                    acc = jnp.where(row >= 0, acc, -1e9 * LOG2E)
                lg.append(acc)
            m = lg[0]
            for w in range(1, W):
                m = jnp.maximum(m, lg[w])
            e = [jnp.exp2(x - m) for x in lg]
            s = e[0]
            for w in range(1, W):
                s = s + e[w]
            inv = 1.0 / s
            for j in range(NP):
                acc = e[0] * vbuf[j, pl.ds(r + HALO, 16), :]
                for w in range(1, W):
                    acc = acc + e[w] * vbuf[j, pl.ds(r + HALO - DIL * w, 16), :]
                obuf[pl.ds(r, 16), j * 128:(j + 1) * 128] = (acc * inv).astype(BF16)

        def a_core(b, s):
            for r in range(s * ASL, (s + 1) * ASL, 16):
                a_core16(b, r, r == 0)

        def a_wo(b):
            xres[b] = xres[b] + lax.dot_general(wopT[...], obuf[...], NT, preferred_element_type=F32)

        def a_ln2(b, slot):
            xnF[slot] = _ln_T(xres[b]).astype(BF16).T

        hvals = {}

        def f_gu(c):
            xv = xnF[sF]
            g = jnp.dot(xv, wg_v[c], preferred_element_type=F32)
            u = jnp.dot(xv, wu_v[c], preferred_element_type=F32)
            hvals[c] = _gelu_mul(g, u).astype(BF16)

        def f_d(c):
            xres[bF] = xres[bF] + lax.dot_general(wd_v[c], hvals.pop(c), NT, preferred_element_type=F32)

        def cp(i, src, dst):
            return pltpu.make_async_copy(src, dst, sems.at[i])

        @pl.when(n == 0)
        def _():
            cq = cp(0, wqkv_hbm, wqkv_v)
            co = cp(1, wo_hbm, wo_v)
            cq.start()
            co.start()
            cf = []
            for c in range(NC):
                cf.append(cp(2 + 3 * c, wg_hbm.at[:, pl.ds(c * FC, FC)], wg_v.at[c]))
                cf.append(cp(3 + 3 * c, wu_hbm.at[:, pl.ds(c * FC, FC)], wu_v.at[c]))
                cf.append(cp(4 + 3 * c, wdT_hbm.at[:, pl.ds(c * FC, FC)], wd_v.at[c]))
            for x in cf:
                x.start()
            kbuf[...] = jnp.zeros(kbuf.shape, F32)
            vbuf[...] = jnp.zeros(vbuf.shape, F32)
            xres[0] = x0_ref[...].astype(F32)
            a_ln(0)
            r = lax.broadcasted_iota(jnp.int32, (DP, DP), 0)
            cidx = lax.broadcasted_iota(jnp.int32, (DP, DP), 1)
            dd = cidx >> 5
            f_of_c = jnp.where(dd < DH, (cidx & 31) * DH + dd, -1000)
            pm0 = jnp.where(f_of_c == r, 1.0, 0.0).astype(BF16)
            pm1 = jnp.where(f_of_c == r - 64, 1.0, 0.0).astype(BF16)
            cq.wait()
            wqp[0] = jnp.dot(wqkv_v[:, pl.ds(0, DP)], pm0, preferred_element_type=F32).astype(BF16)
            wqp[1] = jnp.dot(wqkv_v[:, pl.ds(512, DP)], pm1, preferred_element_type=F32).astype(BF16)
            wqp[2] = jnp.dot(wqkv_v[:, pl.ds(1152, D)], pm0[:D], preferred_element_type=F32).astype(BF16)
            co.wait()
            wopT[...] = lax.dot_general(wo_v[...], pm0[:D], TN, preferred_element_type=F32).astype(BF16)
            a_q()
            a_kv(0, 1, kbuf)
            a_kv(0, 2, vbuf)
            for s in range(NS):
                a_core(0, s)
            a_wo(0)
            a_ln2(0, 0)
            for x in cf:
                x.wait()

        @pl.when(n + 1 < NB)
        def _():
            xres[n + 1] = x1_ref[...].astype(F32)

        bA = (n + 1) & (NB - 1)
        sA = (n + 1) & 1
        tasks = {
            'ln': lambda: a_ln(bA),
            'q': a_q,
            'k': lambda: a_kv(bA, 1, kbuf),
            'v': lambda: a_kv(bA, 2, vbuf),
            'wo': lambda: a_wo(bA),
            'ln2': lambda: a_ln2(bA, sA),
        }
        for s in range(NS):
            tasks['c%d' % s] = functools.partial(a_core, bA, s)
        for c in range(NC):
            tasks['g%d' % c] = functools.partial(f_gu, c)
            tasks['d%d' % c] = functools.partial(f_d, c)
        for t in plan:
            tasks.pop(t)()
        assert not tasks, tasks.keys()
        out_ref[...] = xres[bF].astype(BF16)

    def fn(A_x, A_wqkv, A_wo, B_x, B_w_gate, B_w_up, B_w_down):
        xT = A_x.reshape(S, D).T
        wdT = B_w_down.T
        hbm = pl.BlockSpec(memory_space=pltpu.MemorySpace.HBM)
        out = pl.pallas_call(
            kernel,
            grid=(2 * NB,),
            in_specs=[pl.BlockSpec((D, TM), lambda n: (0, 0)),
                      pl.BlockSpec((D, TM), lambda n: (0, jnp.minimum(n + 1, NB - 1))),
                      hbm, hbm, hbm, hbm, hbm],
            out_specs=pl.BlockSpec((D, TM), lambda n: (0, jnp.maximum(n - NB, 0))),
            out_shape=jax.ShapeDtypeStruct((D, S), BF16),
            scratch_shapes=[
                pltpu.VMEM((D, 3 * D), BF16),
                pltpu.VMEM((D, D), BF16),
                pltpu.VMEM((3, D, DP), BF16),
                pltpu.VMEM((D, DP), BF16),
                pltpu.VMEM((NC, D, FC), BF16),
                pltpu.VMEM((NC, D, FC), BF16),
                pltpu.VMEM((NC, D, FC), BF16),
                pltpu.VMEM((NB, D, TM), F32),
                pltpu.VMEM((TM, D), BF16),
                pltpu.VMEM((2, TM, D), BF16),
                pltpu.VMEM((NP, TM, 128), F32),
                pltpu.VMEM((NP, TM + HALO, 128), F32),
                pltpu.VMEM((NP, TM + HALO, 128), F32),
                pltpu.VMEM((TM, DP), BF16),
                pltpu.SemaphoreType.DMA((2 + 3 * NC,)),
            ],
            compiler_params=pltpu.CompilerParams(
                dimension_semantics=("arbitrary",),
                vmem_limit_bytes=100 * 1024 * 1024,
            ),
        )(xT, xT, A_wqkv, A_wo, B_w_gate, B_w_up, wdT)
        return out.T.reshape(1, S, D)
    return fn


def plan_default(NC, NS):
    p = ['g0', 'ln', 'g1', 'q', 'd0', 'k', 'g2', 'v', 'd1']
    rest = []
    for c in range(3, NC):
        rest += ['g%d' % c, 'd%d' % (c - 1)]
    rest += ['d%d' % (NC - 1)]
    a = ['c%d' % s for s in range(NS)]
    nslots = len(rest) - 3
    out = []
    ai = 0
    for i, t in enumerate(rest[:nslots]):
        out.append(t)
        while ai < len(a) and (ai + 1) * nslots <= (i + 1) * len(a):
            out.append(a[ai]); ai += 1
    out += a[ai:]
    out += ['wo', rest[nslots], 'ln2'] + rest[nslots + 1:]
    return p + out


_TM, _FC, _ASL = 256, 512, 32
_impl = make(_TM, _FC, plan_default(DF // _FC, _TM // _ASL), _ASL)


@jax.jit
def pallas_interleave_layers__sliding_local_dilated__glu_gated_geglu__prompt_kernel(
    A_x, A_wqkv, A_wo, B_x, B_w_gate, B_w_up, B_w_down):
    return _impl(A_x, A_wqkv, A_wo, B_x, B_w_gate, B_w_up, B_w_down)
```

```python
import functools
import contextlib
import numpy as np
import jax
import jax.numpy as jnp
from jax import lax
import jax.experimental.pallas as pl
import jax.experimental.pallas.tpu as pltpu

S, D, DF, H, DH, W, DIL = 2048, 576, 4608, 32, 18, 8, 2
DP = 640
NP = 5
HALO = 16
LOG2E = 1.4426950408889634
QSCALE = float(DH ** -0.5) * LOG2E
F32, BF16, U32 = jnp.float32, jnp.bfloat16, jnp.uint32
NT = (((1,), (1,)), ((), ()))


def _ln_T(xT):
    m = jnp.mean(xT, axis=0, keepdims=True)
    xc = xT - m
    v = jnp.mean(xc * xc, axis=0, keepdims=True)
    return xc * lax.rsqrt(v + 1e-5)


def _gelu_mul(g, u):
    c0 = 0.7978845608028654
    c1 = 0.7978845608028654 * 0.044715
    inner = g * (c0 + c1 * (g * g))
    t = jnp.tanh(inner)
    hg = 0.5 * g
    return (hg + hg * t) * u


def _gather_rows(planes, off2, store):
    for j in range(NP):
        for d2 in range(DH // 2):
            a = planes[j, pl.ds(off2 + d2, 16, stride=DH), :]
            b = planes[j, pl.ds(off2 + d2 + DH // 2, 16, stride=DH), :]
            ev = (a & jnp.uint32(0xFFFF)) | (b << 16)
            od = (a >> 16) | (b & jnp.uint32(0xFFFF0000))
            store(j, 2 * d2, pltpu.bitcast(ev, BF16))
            store(j, 2 * d2 + 1, pltpu.bitcast(od, BF16))


def make(TM=256, FC=512, plan=None, ASL=32, scopes=False, core='c16', hack='', LA=3, FU=1):
    NB = S // TM
    NC = DF // FC
    NS = TM // ASL
    NSL = 1
    while NSL < LA + 1:
        NSL *= 2

    def kernel(x_hbm, wqkv_hbm, wo_hbm, wg_hbm, wu_hbm, wdT_hbm, out_hbm,
               xin, ost, wqkv_v, wo_v, planes, wop, wqpT, wopT, wg_v, wu_v, wd_v,
               xres, xnA, xnF, qbuf, kbuf, vbuf, obuf, wsem, xsem, osem):
        sc = (lambda nm: jax.named_scope(nm)) if scopes else (lambda nm: contextlib.nullcontext())

        def a_ln(b):
            xnA[...] = _ln_T(xres[b]).astype(BF16).T

        def a_q():
            qv = lax.dot_general(xnA[...], wqpT[0], NT, preferred_element_type=F32)
            for j in range(NP):
                qbuf[j] = qv[:, j * 128:(j + 1) * 128] * QSCALE

        def a_kv(b, c, buf, first=False):
            old = [buf[j, pl.ds(TM, HALO), :] for j in range(NP)]
            kv = lax.dot_general(xnA[...], wqpT[c], NT, preferred_element_type=F32)
            for j in range(NP):
                kj = kv[:, j * 128:(j + 1) * 128]
                buf[j, pl.ds(HALO, TM), :] = kj
                rep = jnp.broadcast_to(kj[0:1, :], (HALO, 128))
                buf[j, pl.ds(0, HALO), :] = jnp.where(b == 0, rep, old[j])

        def softmax_w(lg):
            m = lg[0]
            for w in range(1, W):
                m = jnp.maximum(m, lg[w])
            e = [jnp.exp2(x - m) for x in lg]
            s = e[0]
            for w in range(1, W):
                s = s + e[w]
            return e, 1.0 / s

        def a_core16(b, r, masked):
            q = [qbuf[j, pl.ds(r, 16), :] for j in range(NP)]
            lg = []
            for w in range(W):
                o = HALO - DIL * w
                acc = q[0] * kbuf[0, pl.ds(r + o, 16), :]
                for j in range(1, NP):
                    acc = acc + q[j] * kbuf[j, pl.ds(r + o, 16), :]
                acc = acc + pltpu.roll(acc, 64, 1)
                acc = acc + pltpu.roll(acc, 32, 1)
                if masked and w > 0:
                    row = lax.broadcasted_iota(jnp.int32, (16, 128), 0) + (b * TM + r - DIL * w)
                    acc = jnp.where(row >= 0, acc, -1e9 * LOG2E)
                lg.append(acc)
            e, inv = softmax_w(lg)
            for j in range(NP):
                acc = e[0] * vbuf[j, pl.ds(r + HALO, 16), :]
                for w in range(1, W):
                    acc = acc + e[w] * vbuf[j, pl.ds(r + HALO - DIL * w, 16), :]
                obuf[pl.ds(r, 16), j * 128:(j + 1) * 128] = (acc * inv).astype(BF16)

        def a_core16s(b, r, masked):
            G = 2
            cache = {}

            def ld(buf, nm, j, off):
                key = (nm, j, off)
                if key not in cache:
                    cache[key] = buf[j, pl.ds(off, 8), :]
                return cache[key]
            lg = [[None] * W for _ in range(G)]
            for j in range(NP):
                for g in range(G):
                    qj = qbuf[j, pl.ds(r + 8 * g, 8), :]
                    for w in range(W):
                        p = qj * ld(kbuf, 'k', j, r + 8 * g + HALO - DIL * w)
                        lg[g][w] = p if j == 0 else lg[g][w] + p
            es, invs = [], []
            for g in range(G):
                for w in range(W):
                    acc = lg[g][w]
                    acc = acc + pltpu.roll(acc, 64, 1)
                    acc = acc + pltpu.roll(acc, 32, 1)
                    if masked and w > 0:
                        row = lax.broadcasted_iota(jnp.int32, (8, 128), 0) + (b * TM + r + 8 * g - DIL * w)
                        acc = jnp.where(row >= 0, acc, -1e9 * LOG2E)
                    lg[g][w] = acc
                e, inv = softmax_w(lg[g])
                es.append(e)
                invs.append(inv)
            for j in range(NP):
                outs = []
                for g in range(G):
                    acc = es[g][0] * ld(vbuf, 'v', j, r + 8 * g + HALO)
                    for w in range(1, W):
                        acc = acc + es[g][w] * ld(vbuf, 'v', j, r + 8 * g + HALO - DIL * w)
                    outs.append(acc * invs[g])
                obuf[pl.ds(r, 16), j * 128:(j + 1) * 128] = jnp.concatenate(outs, axis=0).astype(BF16)

        core_fn = {'c16': a_core16, 'c16s': a_core16s}[core]

        def a_core(b, s, first):
            for r in range(s * ASL, (s + 1) * ASL, 16):
                core_fn(b, r, r == 0)

        def a_wo(b):
            xres[b] = xres[b] + lax.dot_general(wopT[...], obuf[...], NT, preferred_element_type=F32)

        def a_ln2(b, slot):
            xnF[slot] = _ln_T(xres[b]).astype(BF16).T

        def cw(i, src, dst):
            return pltpu.make_async_copy(src, dst, wsem.at[i])

        def c_qkv():
            return cw(0, wqkv_hbm, wqkv_v)

        def c_wo():
            return cw(1, wo_hbm, wo_v)

        def c_g(c):
            return cw(2 + 3 * c, wg_hbm.at[:, pl.ds(c * FC, FC)], wg_v.at[c])

        def c_u(c):
            return cw(3 + 3 * c, wu_hbm.at[:, pl.ds(c * FC, FC)], wu_v.at[c])

        def c_d(c):
            return cw(4 + 3 * c, wdT_hbm.at[:, pl.ds(c * FC, FC)], wd_v.at[c])

        def c_x(b):
            return pltpu.make_async_copy(x_hbm.at[:, pl.ds(b * TM, TM)], xin.at[b], xsem.at[b])

        def c_o(b):
            return pltpu.make_async_copy(ost.at[b], out_hbm.at[:, pl.ds(pl.multiple_of(b * TM, TM), TM)], osem.at[b])

        def f_tasks(n):
            bF = n & (NB - 1)
            sF = n & (NSL - 1)
            hvals = {}

            def f_gu(c):
                xv = xnF[sF]
                g = jnp.dot(xv, wg_v[c], preferred_element_type=F32)
                u = jnp.dot(xv, wu_v[c], preferred_element_type=F32)
                hvals[c] = _gelu_mul(g, u).astype(BF16)

            def f_d(c):
                xres[bF] = xres[bF] + lax.dot_general(wd_v[c], hvals.pop(c), NT, preferred_element_type=F32)

            tasks = {}
            for c in range(NC):
                tasks['g%d' % c] = functools.partial(f_gu, c)
                tasks['d%d' % c] = functools.partial(f_d, c)
            return tasks

        def a_tasks(m):
            bA = m & (NB - 1)
            sA = m & (NSL - 1)
            tasks = {
                'ln': lambda: a_ln(bA),
                'q': a_q,
                'k': lambda: a_kv(bA, 1, kbuf, False),
                'v': lambda: a_kv(bA, 2, vbuf, False),
                'wo': lambda: a_wo(bA),
                'ln2': lambda: a_ln2(bA, sA),
            }
            for s in range(NS):
                tasks['c%d' % s] = functools.partial(a_core, bA, s, False)
            return tasks

        def load_x(m):
            c_x(m).wait()
            xres[m] = xin[m].astype(F32)

        def finish_f(n):
            bF = n & (NB - 1)
            ost[bF] = xres[bF].astype(BF16)

            @pl.when(n >= NB)
            def _():
                c_o(bF).start()

        with sc('prologue'):
            c_x(0).start()
            c_qkv().start()
            c_wo().start()
            for b in range(1, LA):
                c_x(b).start()
            kbuf[...] = jnp.zeros(kbuf.shape, F32)
            vbuf[...] = jnp.zeros(vbuf.shape, F32)
            c_qkv().wait()
            for c in range(NC):
                c_g(c).start()
                c_u(c).start()
                c_d(c).start()
            for b in range(LA, NB):
                c_x(b).start()
            for c, (start, off) in enumerate(((0, 0), (512, 64), (1152, 0))):
                width = min(DP, 3 * D - start)
                wt32 = pltpu.bitcast(wqkv_v[:, pl.ds(start, width)].T, U32)
                for j in range(NP):
                    lw = min(128, D - j * 128)
                    planes[j, pl.ds(0, width // 2), pl.ds(0, lw)] = wt32[:, j * 128:j * 128 + lw]

                def st(j, dd, val, c=c):
                    lw = min(128, D - j * 128)
                    wqpT[c, pl.ds(dd * 32, 32), pl.ds(j * 128, lw)] = val[:, :lw]
                _gather_rows(planes, off // 2, st)
                wqpT[c, pl.ds(D, DP - D), :] = jnp.zeros((DP - D, D), BF16)
            c_wo().wait()
            wo32 = pltpu.bitcast(wo_v[...], U32)
            for j in range(NP):
                lw = min(128, D - j * 128)
                planes[j, pl.ds(0, D // 2), pl.ds(0, lw)] = wo32[:, j * 128:j * 128 + lw]

            def st2(j, dd, val):
                lw = min(128, D - j * 128)
                wop[pl.ds(dd * 32, 32), pl.ds(j * 128, lw)] = val[:, :lw]
            _gather_rows(planes, 0, st2)
            wop[pl.ds(D, DP - D), :] = jnp.zeros((DP - D, D), BF16)
            wopT[...] = wop[...].T

        with sc('aonly'):
            def abody(m, carry):
                load_x(m)
                t = a_tasks(m)
                for nm in ['ln', 'q', 'k', 'v'] + ['c%d' % s for s in range(NS)] + ['wo', 'ln2']:
                    t[nm]()
                return carry
            lax.fori_loop(0, LA, abody, 0)
            for c in range(NC):
                c_g(c).wait()
                c_u(c).wait()
                c_d(c).wait()

        def body(n, carry):
            @pl.when(n + LA < NB)
            def _():
                load_x(n + LA)
            with sc('main'):
                t = f_tasks(n)
                t.update(a_tasks(n + LA))
                for nm in plan:
                    t.pop(nm)()
                assert not t
                finish_f(n)
            return carry
        lax.fori_loop(0, 2 * NB - LA, body, 0)

        with sc('last'):
            def fbody(n, carry):
                bF = n & (NB - 1)
                sF = n & (NSL - 1)

                def cbody(cc, carry2):
                    xv = xnF[sF]
                    hs = []
                    for i in range(FU):
                        c = cc * FU + i
                        g = jnp.dot(xv, wg_v[c], preferred_element_type=F32)
                        u = jnp.dot(xv, wu_v[c], preferred_element_type=F32)
                        hs.append(_gelu_mul(g, u).astype(BF16))
                        if i > 0:
                            xres[bF] = xres[bF] + lax.dot_general(wd_v[c - 1], hs[i - 1], NT, preferred_element_type=F32)
                    xres[bF] = xres[bF] + lax.dot_general(wd_v[cc * FU + FU - 1], hs[FU - 1], NT, preferred_element_type=F32)
                    return carry2
                lax.fori_loop(0, NC // FU, cbody, 0)
                finish_f(n)
                return carry
            lax.fori_loop(2 * NB - LA, 2 * NB, fbody, 0)
            for b in range(NB):
                c_o(b).wait()

    def fn(A_x, A_wqkv, A_wo, B_x, B_w_gate, B_w_up, B_w_down):
        xT = A_x.reshape(S, D).T
        wdT = B_w_down.T
        hbm = pl.BlockSpec(memory_space=pltpu.MemorySpace.HBM)
        out = pl.pallas_call(
            kernel,
            in_specs=[hbm] * 6,
            out_specs=hbm,
            out_shape=jax.ShapeDtypeStruct((D, S), BF16),
            scratch_shapes=[
                pltpu.VMEM((NB, D, TM), BF16),
                pltpu.VMEM((NB, D, TM), BF16),
                pltpu.VMEM((D, 3 * D), BF16),
                pltpu.VMEM((D, D), BF16),
                pltpu.VMEM((NP, 320, 128), U32),
                pltpu.VMEM((DP, D), BF16),
                pltpu.VMEM((3, DP, D), BF16),
                pltpu.VMEM((D, DP), BF16),
                pltpu.VMEM((NC, D, FC), BF16),
                pltpu.VMEM((NC, D, FC), BF16),
                pltpu.VMEM((NC, D, FC), BF16),
                pltpu.VMEM((NB, D, TM), F32),
                pltpu.VMEM((TM, D), BF16),
                pltpu.VMEM((NSL, TM, D), BF16),
                pltpu.VMEM((NP, TM, 128), F32),
                pltpu.VMEM((NP, TM + HALO, 128), F32),
                pltpu.VMEM((NP, TM + HALO, 128), F32),
                pltpu.VMEM((TM, DP), BF16),
                pltpu.SemaphoreType.DMA((2 + 3 * NC,)),
                pltpu.SemaphoreType.DMA((NB,)),
                pltpu.SemaphoreType.DMA((NB,)),
            ],
            compiler_params=pltpu.CompilerParams(vmem_limit_bytes=100 * 1024 * 1024),
        )(xT, A_wqkv, A_wo, B_w_gate, B_w_up, wdT)
        return out.T.reshape(1, S, D)
    return fn


def plan_default(NC, NS):
    p = ['g0', 'ln', 'g1', 'q', 'd0', 'k', 'g2', 'v', 'd1']
    rest = []
    for c in range(3, NC):
        rest += ['g%d' % c, 'd%d' % (c - 1)]
    rest += ['d%d' % (NC - 1)]
    a = ['c%d' % s for s in range(NS)]
    nslots = len(rest) - 3
    out = []
    ai = 0
    for i, t in enumerate(rest[:nslots]):
        out.append(t)
        while ai < len(a) and (ai + 1) * nslots <= (i + 1) * len(a):
            out.append(a[ai]); ai += 1
    out += a[ai:]
    out += ['wo', rest[nslots], 'ln2'] + rest[nslots + 1:]
    return p + out


_impl = make(256, 512, plan_default(9, 8), 32, LA=3, FU=3)


@jax.jit
def pallas_interleave_layers__sliding_local_dilated__glu_gated_geglu__prompt_kernel(
    A_x, A_wqkv, A_wo, B_x, B_w_gate, B_w_up, B_w_down):
    return _impl(A_x, A_wqkv, A_wo, B_x, B_w_gate, B_w_up, B_w_down)
```

```python
import functools
import contextlib
import numpy as np
import jax
import jax.numpy as jnp
from jax import lax
import jax.experimental.pallas as pl
import jax.experimental.pallas.tpu as pltpu

S, D, DF, H, DH, W, DIL = 2048, 576, 4608, 32, 18, 8, 2
DP = 640
NP = 5
TM = 256
NB = S // TM
SB = 128
XH = 112
XR = XH + SB
LOG2E = 1.4426950408889634
QSCALE = float(DH ** -0.5) * LOG2E
F32, BF16, U32 = jnp.float32, jnp.bfloat16, jnp.uint32
NT = (((1,), (1,)), ((), ()))


def _ln_T(xT):
    m = jnp.mean(xT, axis=0, keepdims=True)
    xc = xT - m
    v = jnp.mean(xc * xc, axis=0, keepdims=True)
    return xc * lax.rsqrt(v + 1e-5)


def _gelu_mul(g, u):
    c0 = 0.7978845608028654
    c1 = 0.7978845608028654 * 0.044715
    inner = g * (c0 + c1 * (g * g))
    t = jnp.tanh(inner)
    hg = 0.5 * g
    return (hg + hg * t) * u


def _perm_tokens(xbf):
    x32 = pltpu.bitcast(xbf, U32)
    l = lax.broadcasted_iota(jnp.int32, (D // 2, 128), 1)
    idx = 16 * ((l >> 1) & 7) + 2 * (l >> 4) + (l & 1)
    parts = [jnp.take_along_axis(x32[:, t * 128:(t + 1) * 128], idx, axis=1) for t in range(TM // 128)]
    return pltpu.bitcast(jnp.concatenate(parts, axis=1), BF16)


def _perm_tokens_f32(x):
    l = lax.broadcasted_iota(jnp.int32, (D, 128), 1)
    idx = 16 * ((l >> 1) & 7) + 2 * (l >> 4) + (l & 1)
    parts = [jnp.take_along_axis(x[:, t * 128:(t + 1) * 128], idx, axis=1) for t in range(TM // 128)]
    return jnp.concatenate(parts, axis=1)


def _gather_rows(planes, off2, store):
    for j in range(NP):
        for d2 in range(DH // 2):
            a = planes[j, pl.ds(off2 + d2, 16, stride=DH), :]
            b = planes[j, pl.ds(off2 + d2 + DH // 2, 16, stride=DH), :]
            ev = (a & jnp.uint32(0xFFFF)) | (b << 16)
            od = (a >> 16) | (b & jnp.uint32(0xFFFF0000))
            store(j, 2 * d2, pltpu.bitcast(ev, BF16))
            store(j, 2 * d2 + 1, pltpu.bitcast(od, BF16))


def make(FC=512, plan=None, scopes=False, LA=3, FU=3, aplan=None, hack='', chain=0, chainA=0, finmode=0):
    NC = DF // FC
    NSL = 1
    while NSL < LA + 1:
        NSL *= 2
    GROUPS = [(sb, j) for sb in range(TM // SB) for j in range(8)]

    def kernel(x_hbm, wqkv_hbm, wo_hbm, wg_hbm, wu_hbm, wdT_hbm, out_hbm,
               xin, ost, wqkv_v, wo_v, planes, wop, wqT, wopT, wg_v, wu_v, wd_v,
               xmid, xout, xa, facc, xnA, xnF, qbuf, kext, vext, obuf, wsem, xsem, osem):
        sc = (lambda nm: jax.named_scope(nm)) if scopes else (lambda nm: contextlib.nullcontext())

        def a_ln(m):
            b = m & (NB - 1)
            x0 = xin[b].astype(F32)
            x = jnp.where(m < NB, x0, xout[b])
            xa[...] = x
            xnA[...] = _perm_tokens(_ln_T(x).astype(BF16)).T

        def mm(r0, nt):
            return lax.dot_general(xnA[...], wqT[pl.ds(r0, nt * 128), :], NT, preferred_element_type=F32)

        def put_ext(m, ext, j, val):
            b = m & (NB - 1)
            cur = m & 1
            prv = 1 - cur
            for sb in range(TM // SB):
                ext[cur, j, pl.ds(sb * XR + XH, SB), :] = val[sb * SB:(sb + 1) * SB, :]
            rep = jnp.broadcast_to(val[0:1, :], (8, 128))
            row = lax.broadcasted_iota(jnp.int32, (8, 128), 0)
            top2 = row < 2
            for dl in range(1, 8):
                ph = ext[prv, j, pl.ds((TM // SB - 1) * XR + XH + 16 * dl + 8, 8), :]
                ph = pltpu.roll(jnp.where(b == 0, rep, ph), 2, 0)
                for sb in range(TM // SB):
                    lo = pltpu.roll(val[sb * SB + 16 * dl: sb * SB + 16 * dl + 8, :], 2, 0)
                    hi = pltpu.roll(val[sb * SB + 16 * dl + 8: sb * SB + 16 * dl + 16, :], 2, 0)
                    ext[cur, j, pl.ds(sb * XR + 16 * (dl - 1), 8), :] = jnp.where(top2, ph, lo)
                    ext[cur, j, pl.ds(sb * XR + 16 * (dl - 1) + 8, 8), :] = jnp.where(top2, lo, hi)
                    ph = hi

        def a_q():
            qv = mm(0, 4)
            for j in range(4):
                qbuf[j] = qv[:, j * 128:(j + 1) * 128] * QSCALE

        def a_kv(m, c, ext):
            kv = mm(512 * c, 4)
            for j in range(4):
                put_ext(m, ext, j, kv[:, j * 128:(j + 1) * 128])

        def a_r(m):
            rv = mm(1536, 2)
            ta = rv[:, 0:128]
            lane = lax.broadcasted_iota(jnp.int32, (TM, 128), 1)
            qbuf[4] = jnp.where(lane < 64, ta * QSCALE, 0.0)
            put_ext(m, kext, 4, pltpu.roll(ta, 64, 1))
            put_ext(m, vext, 4, rv[:, 128:256])

        def a_core(m, sb, jg, links=None, chain=0):
            b = m & (NB - 1)
            cur = m & 1
            r = sb * SB + 16 * jg
            q = [qbuf[j, pl.ds(r, 16), :] for j in range(NP)]
            if links is not None and len(links) >= chain:
                z = links.pop(0)
                q = [pltpu.bitcast(pltpu.bitcast(x, U32) | z, F32) for x in q]
            lg = []
            for w in range(W):
                o = sb * XR + 16 * (jg - w + 7)
                acc = q[0] * kext[cur, 0, pl.ds(o, 16), :]
                for j in range(1, NP):
                    acc = acc + q[j] * kext[cur, j, pl.ds(o, 16), :]
                if 'R' not in hack:
                    acc = acc + pltpu.roll(acc, 64, 1)
                    acc = acc + pltpu.roll(acc, 32, 1)
                if sb == 0 and w > jg:
                    row = lax.broadcasted_iota(jnp.int32, (16, 128), 0)
                    acc = jnp.where(jnp.logical_and(row < 2, b == 0), -1e9 * LOG2E, acc)
                lg.append(acc)
            mx = lg[0]
            for w in range(1, W):
                mx = jnp.maximum(mx, lg[w])
            e = [jnp.exp2(x - mx) if 'E' not in hack else (x - mx) for x in lg]
            s = e[0]
            for w in range(1, W):
                s = s + e[w]
            inv = 1.0 / s
            if links is not None:
                links.append(pltpu.bitcast(inv, U32) >> 31)
            for j in range(NP):
                acc = e[0] * vext[cur, j, pl.ds(sb * XR + 16 * (jg + 7), 16), :]
                for w in range(1, W):
                    acc = acc + e[w] * vext[cur, j, pl.ds(sb * XR + 16 * (jg - w + 7), 16), :]
                obuf[pl.ds(r, 16), j * 128:(j + 1) * 128] = (acc * inv).astype(BF16)

        def a_wo(m):
            b = m & (NB - 1)
            x1 = xa[...] + _perm_tokens_f32(lax.dot_general(wopT[...], obuf[...], NT, preferred_element_type=F32))
            xa[...] = x1
            xmid[b] = x1

        def a_ln2(m):
            b = m & (NB - 1)
            xnF[m & (NSL - 1)] = _ln_T(xa[...]).astype(BF16).T

        def a_tasks(m, chain):
            tasks = {
                'ln': lambda: a_ln(m),
                'q': a_q,
                'k': lambda: a_kv(m, 1, kext),
                'v': lambda: a_kv(m, 2, vext),
                'r': lambda: a_r(m),
                'wo': lambda: a_wo(m),
                'ln2': lambda: a_ln2(m),
            }
            links = [] if chain else None
            tasks['_links'] = links
            for i, (sb, jg) in enumerate(GROUPS):
                tasks['c%d' % i] = functools.partial(a_core, m, sb, jg, links, chain)
            return tasks

        def f_tasks(n):
            bF = n & (NB - 1)
            sF = n & (NSL - 1)
            hvals = {}

            def f_gu(c):
                xv = xnF[sF]
                g = jnp.dot(xv, wg_v[c], preferred_element_type=F32)
                u = jnp.dot(xv, wu_v[c], preferred_element_type=F32)
                hvals[c] = _gelu_mul(g, u).astype(BF16)

            def f_d(c):
                y = (xmid[bF] if c == 0 else facc[...]) + lax.dot_general(wd_v[c], hvals.pop(c), NT, preferred_element_type=F32)
                if c == NC - 1:
                    xout[bF] = y
                    ost[bF] = y.astype(BF16)
                else:
                    facc[...] = y

            tasks = {}
            for c in range(NC):
                tasks['g%d' % c] = functools.partial(f_gu, c)
                tasks['d%d' % c] = functools.partial(f_d, c)
            return tasks

        def cw(i, src, dst):
            return pltpu.make_async_copy(src, dst, wsem.at[i])

        def c_qkv():
            return cw(0, wqkv_hbm, wqkv_v)

        def c_wo():
            return cw(1, wo_hbm, wo_v)

        def c_g(c):
            return cw(2 + 3 * c, wg_hbm.at[:, pl.ds(c * FC, FC)], wg_v.at[c])

        def c_u(c):
            return cw(3 + 3 * c, wu_hbm.at[:, pl.ds(c * FC, FC)], wu_v.at[c])

        def c_d(c):
            return cw(4 + 3 * c, wdT_hbm.at[:, pl.ds(c * FC, FC)], wd_v.at[c])

        def c_x(b):
            return pltpu.make_async_copy(x_hbm.at[:, pl.ds(pl.multiple_of(b * TM, TM), TM)], xin.at[b], xsem.at[b])

        def c_o(b):
            return pltpu.make_async_copy(ost.at[b], out_hbm.at[:, pl.ds(pl.multiple_of(b * TM, TM), TM)], osem.at[b])

        def stage_out(n):
            bF = n & (NB - 1)
            ost[bF] = xout[bF].astype(BF16)

        def finish_f(n):
            bF = n & (NB - 1)
            ost[bF] = xout[bF].astype(BF16)

            @pl.when(n >= NB)
            def _():
                c_o(bF).start()

        with sc('prologue'):
            c_x(0).start()
            c_qkv().start()
            c_wo().start()
            for b in range(1, LA):
                c_x(b).start()
            kext[...] = jnp.zeros(kext.shape, F32)
            vext[...] = jnp.zeros(vext.shape, F32)
            xout[...] = jnp.zeros(xout.shape, F32)
            wqT[pl.ds(1728, 64), :] = jnp.zeros((64, D), BF16)
            wop[pl.ds(D, DP - D), :] = jnp.zeros((DP - D, D), BF16)
            c_qkv().wait()
            for c in range(NC):
                c_g(c).start()
                c_u(c).start()
                c_d(c).start()
            for b in range(LA, NB):
                c_x(b).start()
            for c, (start, off) in enumerate(((0, 0), (512, 64), (1152, 0))):
                width = min(DP, 3 * D - start)
                wt32 = pltpu.bitcast(wqkv_v[:, pl.ds(start, width)].T, U32)
                for j in range(NP):
                    lw = min(128, D - j * 128)
                    planes[j, pl.ds(0, width // 2), pl.ds(0, lw)] = wt32[:, j * 128:j * 128 + lw]

                def st(j, dd, val, c=c):
                    lw = min(128, D - j * 128)
                    r0 = c * 512 + 32 * dd if dd < 16 else 1536 + 64 * c + 32 * (dd - 16)
                    wqT[pl.ds(r0, 32), pl.ds(j * 128, lw)] = val[:, :lw]
                _gather_rows(planes, off // 2, st)
            c_wo().wait()
            wo32 = pltpu.bitcast(wo_v[...], U32)
            for j in range(NP):
                lw = min(128, D - j * 128)
                planes[j, pl.ds(0, D // 2), pl.ds(0, lw)] = wo32[:, j * 128:j * 128 + lw]

            def st2(j, dd, val):
                lw = min(128, D - j * 128)
                wop[pl.ds(dd * 32, 32), pl.ds(j * 128, lw)] = val[:, :lw]
            _gather_rows(planes, 0, st2)
            wopT[...] = wop[...].T

        with sc('aonly'):
            def abody(m, carry):
                c_x(m).wait()
                t = a_tasks(m, chainA)
                t.pop('_links')
                for nm in (aplan or (['ln', 'q', 'k', 'r', 'v'] + ['c%d' % i for i in range(len(GROUPS))] + ['wo', 'ln2'])):
                    t.pop(nm)()
                assert not t
                return carry
            lax.fori_loop(0, LA, abody, 0)
            for c in range(NC):
                c_g(c).wait()
                c_u(c).wait()
                c_d(c).wait()

        def body(n, carry):
            @pl.when(n + LA < NB)
            def _():
                c_x(n + LA).wait()
            with sc('main'):
                t = f_tasks(n)
                t.update(a_tasks(n + LA, chain))
                t.pop('_links')
                for nm in plan:
                    t.pop(nm)()
                assert not t

            @pl.when(n >= NB)
            def _():
                c_o(n & (NB - 1)).start()
            return carry
        lax.fori_loop(0, 2 * NB - LA, body, 0)

        with sc('last'):
            def fbody(n, carry):
                bF = n & (NB - 1)
                sF = n & (NSL - 1)

                facc[...] = xmid[bF]

                def cbody(cc, carry2):
                    xv = xnF[sF]
                    hs = []
                    for i in range(FU):
                        c = cc * FU + i
                        g = jnp.dot(xv, wg_v[c], preferred_element_type=F32)
                        u = jnp.dot(xv, wu_v[c], preferred_element_type=F32)
                        hs.append(_gelu_mul(g, u).astype(BF16))
                        if i > 0:
                            facc[...] += lax.dot_general(wd_v[c - 1], hs[i - 1], NT, preferred_element_type=F32)
                    facc[...] += lax.dot_general(wd_v[cc * FU + FU - 1], hs[FU - 1], NT, preferred_element_type=F32)
                    return carry2
                lax.fori_loop(0, NC // FU, cbody, 0)
                xout[bF] = facc[...]
                finish_f(n)
                return carry
            lax.fori_loop(2 * NB - LA, 2 * NB, fbody, 0)
            for b in range(NB):
                c_o(b).wait()

    def fn(A_x, A_wqkv, A_wo, B_x, B_w_gate, B_w_up, B_w_down):
        xT = A_x.reshape(S, D).T
        wdT = B_w_down.T
        hbm = pl.BlockSpec(memory_space=pltpu.MemorySpace.HBM)
        out = pl.pallas_call(
            kernel,
            in_specs=[hbm] * 6,
            out_specs=hbm,
            out_shape=jax.ShapeDtypeStruct((D, S), BF16),
            scratch_shapes=[
                pltpu.VMEM((NB, D, TM), BF16),
                pltpu.VMEM((NB, D, TM), BF16),
                pltpu.VMEM((D, 3 * D), BF16),
                pltpu.VMEM((D, D), BF16),
                pltpu.VMEM((NP, 320, 128), U32),
                pltpu.VMEM((DP, D), BF16),
                pltpu.VMEM((1792, D), BF16),
                pltpu.VMEM((D, DP), BF16),
                pltpu.VMEM((NC, D, FC), BF16),
                pltpu.VMEM((NC, D, FC), BF16),
                pltpu.VMEM((NC, D, FC), BF16),
                pltpu.VMEM((NB, D, TM), F32),
                pltpu.VMEM((NB, D, TM), F32),
                pltpu.VMEM((D, TM), F32),
                pltpu.VMEM((D, TM), F32),
                pltpu.VMEM((TM, D), BF16),
                pltpu.VMEM((NSL, TM, D), BF16),
                pltpu.VMEM((NP, TM, 128), F32),
                pltpu.VMEM((2, NP, 2 * XR + 8, 128), F32),
                pltpu.VMEM((2, NP, 2 * XR + 8, 128), F32),
                pltpu.VMEM((TM, DP), BF16),
                pltpu.SemaphoreType.DMA((2 + 3 * NC,)),
                pltpu.SemaphoreType.DMA((NB,)),
                pltpu.SemaphoreType.DMA((NB,)),
            ],
            compiler_params=pltpu.CompilerParams(vmem_limit_bytes=100 * 1024 * 1024),
        )(xT, A_wqkv, A_wo, B_w_gate, B_w_up, wdT)
        return out.T.reshape(1, S, D)
    return fn


def plan_default(NC=9, NS=16, tail=3):
    p = ['g0', 'ln', 'g1', 'q', 'd0', 'k', 'g2', 'r', 'v', 'd1']
    rest = []
    for c in range(3, NC):
        rest += ['g%d' % c, 'd%d' % (c - 1)]
    rest += ['d%d' % (NC - 1)]
    a = ['c%d' % s for s in range(NS)]
    nslots = len(rest) - tail
    out = []
    ai = 0
    for i, t in enumerate(rest[:nslots]):
        out.append(t)
        while ai < len(a) and (ai + 1) * nslots <= (i + 1) * len(a):
            out.append(a[ai]); ai += 1
    out += a[ai:]
    out += ['wo', rest[nslots], 'ln2'] + rest[nslots + 1:]
    return p + out


def mkplan(pos, NC=9):
    F = ['g0']
    for c in range(1, NC):
        F += ['g%d' % c, 'd%d' % (c - 1)]
    F += ['d%d' % (NC - 1)]
    order = ['ln', 'q', 'k', 'r', 'v'] + ['c%d' % i for i in range(16)] + ['wo', 'ln2']
    out = []
    for i in range(len(F) + 1):
        for a in order:
            if pos[a] == i:
                out.append(a)
        if i < len(F):
            out.append(F[i])
    return out


def P(ln=1, q=2, k=3, r=4, v=4, c0=5, c1=14, wo=15, ln2=16):
    pos = dict(ln=ln, q=q, k=k, r=r, v=v, wo=wo, ln2=ln2)
    for i in range(16):
        pos['c%d' % i] = c0 + ((c1 - c0 + 1) * i) // 16
    return mkplan(pos)


def ins(plan, task, before):
    p = list(plan)
    p.insert(p.index(before), task)
    return p


_impl = make(512, P(), LA=3, chain=1, chainA=3)


@jax.jit
def pallas_interleave_layers__sliding_local_dilated__glu_gated_geglu__prompt_kernel(
    A_x, A_wqkv, A_wo, B_x, B_w_gate, B_w_up, B_w_down):
    return _impl(A_x, A_wqkv, A_wo, B_x, B_w_gate, B_w_up, B_w_down)
```

```python
import functools
import contextlib
import numpy as np
import jax
import jax.numpy as jnp
from jax import lax
import jax.experimental.pallas as pl
import jax.experimental.pallas.tpu as pltpu

S, D, DF, H, DH, W, DIL = 2048, 576, 4608, 32, 18, 8, 2
DP = 640
NP = 5
TM = 256
NB = S // TM
SB = 128
XH = 112
XR = XH + SB
LOG2E = 1.4426950408889634
QSCALE = float(DH ** -0.5) * LOG2E
F32, BF16, U32 = jnp.float32, jnp.bfloat16, jnp.uint32
NT = (((1,), (1,)), ((), ()))


def _ln_T(xT):
    m = jnp.mean(xT, axis=0, keepdims=True)
    xc = xT - m
    v = jnp.mean(xc * xc, axis=0, keepdims=True)
    return xc * lax.rsqrt(v + 1e-5)


def _gelu_mul(g, u):
    c0 = 0.7978845608028654
    c1 = 0.7978845608028654 * 0.044715
    inner = g * (c0 + c1 * (g * g))
    t = jnp.tanh(inner)
    hg = 0.5 * g
    return (hg + hg * t) * u


def _perm_tokens(xbf):
    x32 = pltpu.bitcast(xbf, U32)
    l = lax.broadcasted_iota(jnp.int32, (D // 2, 128), 1)
    idx = 16 * ((l >> 1) & 7) + 2 * (l >> 4) + (l & 1)
    parts = [jnp.take_along_axis(x32[:, t * 128:(t + 1) * 128], idx, axis=1) for t in range(TM // 128)]
    return pltpu.bitcast(jnp.concatenate(parts, axis=1), BF16)


def _perm_tokens_f32(x):
    l = lax.broadcasted_iota(jnp.int32, (D, 128), 1)
    idx = 16 * ((l >> 1) & 7) + 2 * (l >> 4) + (l & 1)
    parts = [jnp.take_along_axis(x[:, t * 128:(t + 1) * 128], idx, axis=1) for t in range(TM // 128)]
    return jnp.concatenate(parts, axis=1)


def _gather_rows(planes, off2, store):
    for j in range(NP):
        for d2 in range(DH // 2):
            a = planes[j, pl.ds(off2 + d2, 16, stride=DH), :]
            b = planes[j, pl.ds(off2 + d2 + DH // 2, 16, stride=DH), :]
            ev = (a & jnp.uint32(0xFFFF)) | (b << 16)
            od = (a >> 16) | (b & jnp.uint32(0xFFFF0000))
            store(j, 2 * d2, pltpu.bitcast(ev, BF16))
            store(j, 2 * d2 + 1, pltpu.bitcast(od, BF16))


def make(FC=512, plan=None, scopes=False, LA=3, FU=3, aplan=None, hack='', chain=0, chainA=0, GSTART=2):
    NC = DF // FC
    NSL = 1
    while NSL < LA + 1:
        NSL *= 2
    GROUPS = [(sb, j) for sb in range(TM // SB) for j in range(8)]

    def kernel(x_hbm, wqkv_hbm, wo_hbm, wg_hbm, wu_hbm, wdT_hbm, out_hbm,
               xin, ost, wqkv_v, wo_v, planes, wop, wqT, wopT, wg_v, wu_v, wd_v,
               xmid, xout, xa, facc, xnA, xnF, qbuf, kext, vext, obuf, wsem, xsem, osem):
        sc = (lambda nm: jax.named_scope(nm)) if scopes else (lambda nm: contextlib.nullcontext())

        def a_ln(m):
            b = m & (NB - 1)
            x0 = xin[b].astype(F32)
            x = jnp.where(m < NB, x0, xout[b])
            xa[...] = x
            xnA[...] = _perm_tokens(_ln_T(x).astype(BF16)).T

        def mm(r0, nt):
            return lax.dot_general(xnA[...], wqT[pl.ds(r0, nt * 128), :], NT, preferred_element_type=F32)

        def put_ext(m, ext, j, val):
            b = m & (NB - 1)
            cur = m & 1
            prv = 1 - cur
            for sb in range(TM // SB):
                ext[cur, j, pl.ds(sb * XR + XH, SB), :] = val[sb * SB:(sb + 1) * SB, :]
            rep = jnp.broadcast_to(val[0:1, :], (8, 128))
            row = lax.broadcasted_iota(jnp.int32, (8, 128), 0)
            top2 = row < 2
            for dl in range(1, 8):
                ph = ext[prv, j, pl.ds((TM // SB - 1) * XR + XH + 16 * dl + 8, 8), :]
                ph = pltpu.roll(jnp.where(b == 0, rep, ph), 2, 0)
                for sb in range(TM // SB):
                    lo = pltpu.roll(val[sb * SB + 16 * dl: sb * SB + 16 * dl + 8, :], 2, 0)
                    hi = pltpu.roll(val[sb * SB + 16 * dl + 8: sb * SB + 16 * dl + 16, :], 2, 0)
                    ext[cur, j, pl.ds(sb * XR + 16 * (dl - 1), 8), :] = jnp.where(top2, ph, lo)
                    ext[cur, j, pl.ds(sb * XR + 16 * (dl - 1) + 8, 8), :] = jnp.where(top2, lo, hi)
                    ph = hi

        def a_q():
            qv = mm(0, 4)
            for j in range(4):
                qbuf[j] = qv[:, j * 128:(j + 1) * 128] * QSCALE

        def a_kv(m, c, ext):
            kv = mm(512 * c, 4)
            for j in range(4):
                put_ext(m, ext, j, kv[:, j * 128:(j + 1) * 128])

        def a_r(m):
            rv = mm(1536, 2)
            ta = rv[:, 0:128]
            lane = lax.broadcasted_iota(jnp.int32, (TM, 128), 1)
            qbuf[4] = jnp.where(lane < 64, ta * QSCALE, 0.0)
            put_ext(m, kext, 4, pltpu.roll(ta, 64, 1))
            put_ext(m, vext, 4, rv[:, 128:256])

        def a_core(m, sb, jg, links=None, chain=0):
            b = m & (NB - 1)
            cur = m & 1
            r = sb * SB + 16 * jg
            q = [qbuf[j, pl.ds(r, 16), :] for j in range(NP)]
            if links is not None and len(links) >= chain:
                z = links.pop(0)
                q = [pltpu.bitcast(pltpu.bitcast(x, U32) | z, F32) for x in q]
            lg = []
            for w in range(W):
                o = sb * XR + 16 * (jg - w + 7)
                acc = q[0] * kext[cur, 0, pl.ds(o, 16), :]
                for j in range(1, NP):
                    acc = acc + q[j] * kext[cur, j, pl.ds(o, 16), :]
                if 'R' not in hack:
                    acc = acc + pltpu.roll(acc, 64, 1)
                    acc = acc + pltpu.roll(acc, 32, 1)
                if sb == 0 and w > jg:
                    row = lax.broadcasted_iota(jnp.int32, (16, 128), 0)
                    acc = jnp.where(jnp.logical_and(row < 2, b == 0), -1e9 * LOG2E, acc)
                lg.append(acc)
            mx = lg[0]
            for w in range(1, W):
                mx = jnp.maximum(mx, lg[w])
            e = [jnp.exp2(x - mx) if 'E' not in hack else (x - mx) for x in lg]
            s = e[0]
            for w in range(1, W):
                s = s + e[w]
            inv = 1.0 / s
            if links is not None:
                links.append(pltpu.bitcast(inv, U32) >> 31)
            for j in range(NP):
                acc = e[0] * vext[cur, j, pl.ds(sb * XR + 16 * (jg + 7), 16), :]
                for w in range(1, W):
                    acc = acc + e[w] * vext[cur, j, pl.ds(sb * XR + 16 * (jg - w + 7), 16), :]
                obuf[pl.ds(r, 16), j * 128:(j + 1) * 128] = (acc * inv).astype(BF16)

        def a_wo(m):
            b = m & (NB - 1)
            x1 = xa[...] + _perm_tokens_f32(lax.dot_general(wopT[...], obuf[...], NT, preferred_element_type=F32))
            xa[...] = x1
            xmid[b] = x1

        def a_ln2(m):
            b = m & (NB - 1)
            xnF[m & (NSL - 1)] = _ln_T(xa[...]).astype(BF16).T

        def a_tasks(m, chain):
            tasks = {
                'ln': lambda: a_ln(m),
                'q': a_q,
                'k': lambda: a_kv(m, 1, kext),
                'v': lambda: a_kv(m, 2, vext),
                'r': lambda: a_r(m),
                'wo': lambda: a_wo(m),
                'ln2': lambda: a_ln2(m),
            }
            links = [] if chain else None
            tasks['_links'] = links
            for i, (sb, jg) in enumerate(GROUPS):
                tasks['c%d' % i] = functools.partial(a_core, m, sb, jg, links, chain)
            return tasks

        def f_tasks(n):
            bF = n & (NB - 1)
            sF = n & (NSL - 1)
            hvals = {}

            def f_gu(c):
                xv = xnF[sF]
                g = jnp.dot(xv, wg_v[c], preferred_element_type=F32)
                u = jnp.dot(xv, wu_v[c], preferred_element_type=F32)
                hvals[c] = _gelu_mul(g, u).astype(BF16)

            def f_d(c):
                y = (xmid[bF] if c == 0 else facc[...]) + lax.dot_general(wd_v[c], hvals.pop(c), NT, preferred_element_type=F32)
                if c == NC - 1:
                    xout[bF] = y
                    ost[bF] = y.astype(BF16)
                else:
                    facc[...] = y

            tasks = {}
            for c in range(NC):
                tasks['g%d' % c] = functools.partial(f_gu, c)
                tasks['d%d' % c] = functools.partial(f_d, c)
            return tasks

        def cw(i, src, dst):
            return pltpu.make_async_copy(src, dst, wsem.at[i])

        def c_qkv(c):
            lo, hi = ((0, 640), (640, 1152), (1152, 1728))[c]
            return cw(2 + 3 * NC + c, wqkv_hbm.at[:, pl.ds(lo, hi - lo)], wqkv_v.at[:, pl.ds(lo, hi - lo)])

        def c_wo():
            return cw(1, wo_hbm, wo_v)

        def c_g(c):
            return cw(2 + 3 * c, wg_hbm.at[:, pl.ds(pl.multiple_of(c * FC, FC), FC)], wg_v.at[c])

        def c_u(c):
            return cw(3 + 3 * c, wu_hbm.at[:, pl.ds(pl.multiple_of(c * FC, FC), FC)], wu_v.at[c])

        def c_d(c):
            return cw(4 + 3 * c, wdT_hbm.at[:, pl.ds(pl.multiple_of(c * FC, FC), FC)], wd_v.at[c])

        def c_x(b):
            return pltpu.make_async_copy(x_hbm.at[:, pl.ds(pl.multiple_of(b * TM, TM), TM)], xin.at[b], xsem.at[b])

        def c_o(b):
            return pltpu.make_async_copy(ost.at[b], out_hbm.at[:, pl.ds(pl.multiple_of(b * TM, TM), TM)], osem.at[b])

        def stage_out(n):
            bF = n & (NB - 1)
            ost[bF] = xout[bF].astype(BF16)

        def finish_f(n):
            bF = n & (NB - 1)
            ost[bF] = xout[bF].astype(BF16)

            @pl.when(n >= NB)
            def _():
                c_o(bF).start()

        def start_group(g):
            for i in range(FU):
                c = g * FU + i
                c_g(c).start()
                c_u(c).start()
                c_d(c).start()

        with sc('prologue'):
            c_x(0).start()
            for c in range(3):
                c_qkv(c).start()
            c_wo().start()
            for b in range(1, LA):
                c_x(b).start()

            def zbody(i, carry):
                kext[i // NP, i % NP] = jnp.zeros(kext.shape[2:], F32)
                vext[i // NP, i % NP] = jnp.zeros(vext.shape[2:], F32)
                return carry
            lax.fori_loop(0, 2 * NP, zbody, 0)

            def zbody2(i, carry):
                xout[i] = jnp.zeros(xout.shape[1:], F32)
                return carry
            lax.fori_loop(0, NB, zbody2, 0)
            wqT[pl.ds(1728, 64), :] = jnp.zeros((64, D), BF16)
            wop[pl.ds(D, DP - D), :] = jnp.zeros((DP - D, D), BF16)
            for c, (start, off) in enumerate(((0, 0), (512, 64), (1152, 0))):
                c_qkv(c).wait()
                if c == GSTART:
                    start_group(0)
                width = min(DP, 3 * D - start)
                wt32 = pltpu.bitcast(wqkv_v[:, pl.ds(start, width)].T, U32)
                for j in range(NP):
                    lw = min(128, D - j * 128)
                    planes[j, pl.ds(0, width // 2), pl.ds(0, lw)] = wt32[:, j * 128:j * 128 + lw]

                def st(j, dd, val, c=c):
                    lw = min(128, D - j * 128)
                    r0 = c * 512 + 32 * dd if dd < 16 else 1536 + 64 * c + 32 * (dd - 16)
                    wqT[pl.ds(r0, 32), pl.ds(j * 128, lw)] = val[:, :lw]
                _gather_rows(planes, off // 2, st)
            c_wo().wait()
            wo32 = pltpu.bitcast(wo_v[...], U32)
            for j in range(NP):
                lw = min(128, D - j * 128)
                planes[j, pl.ds(0, D // 2), pl.ds(0, lw)] = wo32[:, j * 128:j * 128 + lw]

            def st2(j, dd, val):
                lw = min(128, D - j * 128)
                wop[pl.ds(dd * 32, 32), pl.ds(j * 128, lw)] = val[:, :lw]
            _gather_rows(planes, 0, st2)
            wopT[...] = wop[...].T

        with sc('aonly'):
            def abody(m, carry):
                @pl.when(m == LA - 1)
                def _():
                    start_group(1)
                c_x(m).wait()
                t = a_tasks(m, chainA)
                t.pop('_links')
                for nm in (aplan or (['ln', 'q', 'k', 'r', 'v'] + ['c%d' % i for i in range(len(GROUPS))] + ['wo', 'ln2'])):
                    t.pop(nm)()
                assert not t
                return carry
            lax.fori_loop(0, LA, abody, 0)
            for g in range(2, NC // FU):
                start_group(g)
            for b in range(LA, NB):
                c_x(b).start()

        def body(n, carry):
            @pl.when(n + LA - 1 < NB)
            def _():
                c_x(n + LA - 1).wait()
            with sc('main'):
                t = f_tasks(n)
                t.update(a_tasks(n + LA - 1, chain))
                t.pop('_links')
                for nm in plan:
                    t.pop(nm)()
                assert not t

            @pl.when(n >= NB)
            def _():
                c_o(n & (NB - 1)).start()
            return carry

        def fbody(n, carry):
            bF = n & (NB - 1)
            sF = n & (NSL - 1)
            facc[...] = xmid[bF]

            def cbody(cc, carry2):
                @pl.when(n == 0)
                def _():
                    for i in range(FU):
                        c = cc * FU + i
                        c_g(c).wait()
                        c_u(c).wait()
                        c_d(c).wait()
                xv = xnF[sF]
                hs = []
                for i in range(FU):
                    c = cc * FU + i
                    g = jnp.dot(xv, wg_v[c], preferred_element_type=F32)
                    u = jnp.dot(xv, wu_v[c], preferred_element_type=F32)
                    hs.append(_gelu_mul(g, u).astype(BF16))
                    if i > 0:
                        facc[...] += lax.dot_general(wd_v[c - 1], hs[i - 1], NT, preferred_element_type=F32)
                facc[...] += lax.dot_general(wd_v[cc * FU + FU - 1], hs[FU - 1], NT, preferred_element_type=F32)
                return carry2
            lax.fori_loop(0, NC // FU, cbody, 0)
            xout[bF] = facc[...]
            finish_f(n)
            return carry

        def segment(sg, carry):
            with sc('fonly'):
                lax.fori_loop(jnp.where(sg == 0, 0, 2 * NB - LA + 1), jnp.where(sg == 0, 1, 2 * NB), fbody, 0)
            lax.fori_loop(1, jnp.where(sg == 0, 2 * NB - LA + 1, 1), body, 0)
            return carry
        lax.fori_loop(0, 2, segment, 0)
        for b in range(NB):
            c_o(b).wait()

    def fn(A_x, A_wqkv, A_wo, B_x, B_w_gate, B_w_up, B_w_down):
        xT = A_x.reshape(S, D).T
        wdT = B_w_down.T
        hbm = pl.BlockSpec(memory_space=pltpu.MemorySpace.HBM)
        out = pl.pallas_call(
            kernel,
            in_specs=[hbm] * 6,
            out_specs=hbm,
            out_shape=jax.ShapeDtypeStruct((D, S), BF16),
            scratch_shapes=[
                pltpu.VMEM((NB, D, TM), BF16),
                pltpu.VMEM((NB, D, TM), BF16),
                pltpu.VMEM((D, 3 * D), BF16),
                pltpu.VMEM((D, D), BF16),
                pltpu.VMEM((NP, 320, 128), U32),
                pltpu.VMEM((DP, D), BF16),
                pltpu.VMEM((1792, D), BF16),
                pltpu.VMEM((D, DP), BF16),
                pltpu.VMEM((NC, D, FC), BF16),
                pltpu.VMEM((NC, D, FC), BF16),
                pltpu.VMEM((NC, D, FC), BF16),
                pltpu.VMEM((NB, D, TM), F32),
                pltpu.VMEM((NB, D, TM), F32),
                pltpu.VMEM((D, TM), F32),
                pltpu.VMEM((D, TM), F32),
                pltpu.VMEM((TM, D), BF16),
                pltpu.VMEM((NSL, TM, D), BF16),
                pltpu.VMEM((NP, TM, 128), F32),
                pltpu.VMEM((2, NP, 2 * XR + 8, 128), F32),
                pltpu.VMEM((2, NP, 2 * XR + 8, 128), F32),
                pltpu.VMEM((TM, DP), BF16),
                pltpu.SemaphoreType.DMA((5 + 3 * NC,)),
                pltpu.SemaphoreType.DMA((NB,)),
                pltpu.SemaphoreType.DMA((NB,)),
            ],
            compiler_params=pltpu.CompilerParams(vmem_limit_bytes=100 * 1024 * 1024),
        )(xT, A_wqkv, A_wo, B_w_gate, B_w_up, wdT)
        return out.T.reshape(1, S, D)
    return fn


def plan_default(NC=9, NS=16, tail=3):
    p = ['g0', 'ln', 'g1', 'q', 'd0', 'k', 'g2', 'r', 'v', 'd1']
    rest = []
    for c in range(3, NC):
        rest += ['g%d' % c, 'd%d' % (c - 1)]
    rest += ['d%d' % (NC - 1)]
    a = ['c%d' % s for s in range(NS)]
    nslots = len(rest) - tail
    out = []
    ai = 0
    for i, t in enumerate(rest[:nslots]):
        out.append(t)
        while ai < len(a) and (ai + 1) * nslots <= (i + 1) * len(a):
            out.append(a[ai]); ai += 1
    out += a[ai:]
    out += ['wo', rest[nslots], 'ln2'] + rest[nslots + 1:]
    return p + out


def mkplan(pos, NC=9):
    F = ['g0']
    for c in range(1, NC):
        F += ['g%d' % c, 'd%d' % (c - 1)]
    F += ['d%d' % (NC - 1)]
    order = ['ln', 'q', 'k', 'r', 'v'] + ['c%d' % i for i in range(16)] + ['wo', 'ln2']
    out = []
    for i in range(len(F) + 1):
        for a in order:
            if pos[a] == i:
                out.append(a)
        if i < len(F):
            out.append(F[i])
    return out


def P(ln=1, q=2, k=3, r=4, v=4, c0=5, c1=14, wo=15, ln2=16):
    pos = dict(ln=ln, q=q, k=k, r=r, v=v, wo=wo, ln2=ln2)
    for i in range(16):
        pos['c%d' % i] = c0 + ((c1 - c0 + 1) * i) // 16
    return mkplan(pos)


def ins(plan, task, before):
    p = list(plan)
    p.insert(p.index(before), task)
    return p


_impl = make(512, P(), LA=2, chain=1, chainA=3)


@jax.jit
def pallas_interleave_layers__sliding_local_dilated__glu_gated_geglu__prompt_kernel(
    A_x, A_wqkv, A_wo, B_x, B_w_gate, B_w_up, B_w_down):
    return _impl(A_x, A_wqkv, A_wo, B_x, B_w_gate, B_w_up, B_w_down)
```

```python
import functools
import contextlib
import numpy as np
import jax
import jax.numpy as jnp
from jax import lax
import jax.experimental.pallas as pl
import jax.experimental.pallas.tpu as pltpu

S, D, DF, H, DH, W, DIL = 2048, 576, 4608, 32, 18, 8, 2
DP = 640
NP = 5
TM = 256
NB = S // TM
SB = 128
XH = 112
XR = XH + SB
LOG2E = 1.4426950408889634
QSCALE = float(DH ** -0.5) * LOG2E
F32, BF16, U32 = jnp.float32, jnp.bfloat16, jnp.uint32
NT = (((1,), (1,)), ((), ()))


def _ln_T(xT):
    m = jnp.mean(xT, axis=0, keepdims=True)
    xc = xT - m
    v = jnp.mean(xc * xc, axis=0, keepdims=True)
    return xc * lax.rsqrt(v + 1e-5)


def _gelu_mul(g, u):
    c0 = 0.7978845608028654
    c1 = 0.7978845608028654 * 0.044715
    inner = g * (c0 + c1 * (g * g))
    t = jnp.tanh(inner)
    return (g * u) * (t + 1.0)


def _perm_tokens(xbf):
    x32 = pltpu.bitcast(xbf, U32)
    l = lax.broadcasted_iota(jnp.int32, (D // 2, 128), 1)
    idx = 16 * ((l >> 1) & 7) + 2 * (l >> 4) + (l & 1)
    parts = [jnp.take_along_axis(x32[:, t * 128:(t + 1) * 128], idx, axis=1) for t in range(TM // 128)]
    return pltpu.bitcast(jnp.concatenate(parts, axis=1), BF16)


def _perm_tokens_f32(x):
    l = lax.broadcasted_iota(jnp.int32, (D, 128), 1)
    idx = 16 * ((l >> 1) & 7) + 2 * (l >> 4) + (l & 1)
    parts = [jnp.take_along_axis(x[:, t * 128:(t + 1) * 128], idx, axis=1) for t in range(TM // 128)]
    return jnp.concatenate(parts, axis=1)


def _gather_rows(planes, off2, store):
    for j in range(NP):
        for d2 in range(DH // 2):
            a = planes[j, pl.ds(off2 + d2, 16, stride=DH), :]
            b = planes[j, pl.ds(off2 + d2 + DH // 2, 16, stride=DH), :]
            ev = (a & jnp.uint32(0xFFFF)) | (b << 16)
            od = (a >> 16) | (b & jnp.uint32(0xFFFF0000))
            store(j, 2 * d2, pltpu.bitcast(ev, BF16))
            store(j, 2 * d2 + 1, pltpu.bitcast(od, BF16))


def make(FC=512, plan=None, scopes=False, LA=3, FU=3, aplan=None, hack='', chain=0, chainA=0, GSTART=2, only=None, apair=None, LATE=None):
    NC = DF // FC
    NSL = 1
    while NSL < LA + 1:
        NSL *= 2
    GROUPS = [(sb, j) for sb in range(TM // SB) for j in range(8)]

    def kernel(x_hbm, wqkv_hbm, wo_hbm, wg_hbm, wu_hbm, wdT_hbm, out_hbm,
               xin, ost, wqkv_v, wo_v, planes, wop, wqT, wopT, wg_v, wu_v, wd_v,
               xmid, xout, xa, facc, xnA, xnF, qbuf, kext, vext, obuf, wsem, xsem, osem):
        sc = (lambda nm: jax.named_scope(nm)) if scopes else (lambda nm: contextlib.nullcontext())

        def a_ln(m):
            b = m & (NB - 1)
            x0 = xin[b].astype(F32)
            x = jnp.where(m < NB, x0, xout[b])
            xa[m & 1] = x
            xnA[...] = _perm_tokens(_ln_T(x).astype(BF16)).T

        def mm(r0, nt):
            return lax.dot_general(xnA[...], wqT[pl.ds(r0, nt * 128), :], NT, preferred_element_type=F32)

        def put_ext(m, ext, j, val):
            b = m & (NB - 1)
            cur = m & 1
            prv = 1 - cur
            for sb in range(TM // SB):
                ext[cur, j, pl.ds(sb * XR + XH, SB), :] = val[sb * SB:(sb + 1) * SB, :]
            rep = jnp.broadcast_to(val[0:1, :], (8, 128))
            row = lax.broadcasted_iota(jnp.int32, (8, 128), 0)
            top2 = row < 2
            for dl in range(1, 8):
                ph = ext[prv, j, pl.ds((TM // SB - 1) * XR + XH + 16 * dl + 8, 8), :]
                ph = pltpu.roll(jnp.where(b == 0, rep, ph), 2, 0)
                for sb in range(TM // SB):
                    lo = pltpu.roll(val[sb * SB + 16 * dl: sb * SB + 16 * dl + 8, :], 2, 0)
                    hi = pltpu.roll(val[sb * SB + 16 * dl + 8: sb * SB + 16 * dl + 16, :], 2, 0)
                    ext[cur, j, pl.ds(sb * XR + 16 * (dl - 1), 8), :] = jnp.where(top2, ph, lo)
                    ext[cur, j, pl.ds(sb * XR + 16 * (dl - 1) + 8, 8), :] = jnp.where(top2, lo, hi)
                    ph = hi

        def a_q(m):
            qv = mm(0, 4)
            for j in range(4):
                qbuf[m & 1, j] = qv[:, j * 128:(j + 1) * 128] * QSCALE

        def a_kv(m, c, ext):
            kv = mm(512 * c, 4)
            for j in range(4):
                put_ext(m, ext, j, kv[:, j * 128:(j + 1) * 128])

        def a_r(m):
            rv = mm(1536, 2)
            ta = rv[:, 0:128]
            lane = lax.broadcasted_iota(jnp.int32, (TM, 128), 1)
            qbuf[m & 1, 4] = jnp.where(lane < 64, ta * QSCALE, 0.0)
            put_ext(m, kext, 4, pltpu.roll(ta, 64, 1))
            put_ext(m, vext, 4, rv[:, 128:256])

        def a_core(m, sb, jg, links=None, chain=0):
            b = m & (NB - 1)
            cur = m & 1
            r = sb * SB + 16 * jg
            q = [qbuf[cur, j, pl.ds(r, 16), :] for j in range(NP)]
            if links is not None and len(links) >= chain:
                z = links.pop(0)
                q = [pltpu.bitcast(pltpu.bitcast(x, U32) | z, F32) for x in q]
            lg = []
            for w in range(W):
                o = sb * XR + 16 * (jg - w + 7)
                acc = q[0] * kext[cur, 0, pl.ds(o, 16), :]
                for j in range(1, NP):
                    acc = acc + q[j] * kext[cur, j, pl.ds(o, 16), :]
                if 'R' not in hack:
                    acc = acc + pltpu.roll(acc, 64, 1)
                    acc = acc + pltpu.roll(acc, 32, 1)
                if sb == 0 and w > jg:
                    row = lax.broadcasted_iota(jnp.int32, (16, 128), 0)
                    acc = jnp.where(jnp.logical_and(row < 2, b == 0), -1e9 * LOG2E, acc)
                lg.append(acc)
            mx = lg[0]
            for w in range(1, W):
                mx = jnp.maximum(mx, lg[w])
            e = [jnp.exp2(x - mx) if 'E' not in hack else (x - mx) for x in lg]
            s = e[0]
            for w in range(1, W):
                s = s + e[w]
            inv = 1.0 / s
            if links is not None:
                links.append(pltpu.bitcast(inv, U32) >> 31)
            for j in range(NP):
                acc = e[0] * vext[cur, j, pl.ds(sb * XR + 16 * (jg + 7), 16), :]
                for w in range(1, W):
                    acc = acc + e[w] * vext[cur, j, pl.ds(sb * XR + 16 * (jg - w + 7), 16), :]
                obuf[pl.ds(r, 16), j * 128:(j + 1) * 128] = (acc * inv).astype(BF16)

        def a_wo(m):
            b = m & (NB - 1)
            x1 = xa[m & 1] + _perm_tokens_f32(lax.dot_general(wopT[...], obuf[...], NT, preferred_element_type=F32))
            xa[m & 1] = x1
            xmid[b] = x1

        def a_ln2(m):
            b = m & (NB - 1)
            xnF[m & (NSL - 1)] = _ln_T(xa[m & 1]).astype(BF16).T

        def a_tasks(m, chain):
            tasks = {
                'ln': lambda: a_ln(m),
                'q': lambda: a_q(m),
                'k': lambda: a_kv(m, 1, kext),
                'v': lambda: a_kv(m, 2, vext),
                'r': lambda: a_r(m),
                'wo': lambda: a_wo(m),
                'ln2': lambda: a_ln2(m),
            }
            links = [] if chain else None
            tasks['_links'] = links
            for i, (sb, jg) in enumerate(GROUPS):
                tasks['c%d' % i] = functools.partial(a_core, m, sb, jg, links, chain)
            return tasks

        def f_tasks(n):
            bF = n & (NB - 1)
            sF = n & (NSL - 1)
            hvals = {}

            def f_gu(c):
                xv = xnF[sF]
                g = jnp.dot(xv, wg_v[c], preferred_element_type=F32)
                u = jnp.dot(xv, wu_v[c], preferred_element_type=F32)
                hvals[c] = _gelu_mul(g, u).astype(BF16)

            def f_d(c):
                y = lax.dot_general(wd_v[c], hvals.pop(c), NT, preferred_element_type=F32)
                if c > 0:
                    y = facc[...] + y
                if c == NC - 1:
                    y = xmid[bF] + 0.5 * y
                    xout[bF] = y
                    ost[bF] = y.astype(BF16)
                else:
                    facc[...] = y

            tasks = {}
            for c in range(NC):
                tasks['g%d' % c] = functools.partial(f_gu, c)
                tasks['d%d' % c] = functools.partial(f_d, c)
            return tasks

        def cw(i, src, dst):
            return pltpu.make_async_copy(src, dst, wsem.at[i])

        def c_qkv(c):
            lo, hi = ((0, 640), (640, 1152), (1152, 1728))[c]
            return cw(2 + 3 * NC + c, wqkv_hbm.at[:, pl.ds(lo, hi - lo)], wqkv_v.at[:, pl.ds(lo, hi - lo)])

        def c_wo():
            return cw(1, wo_hbm, wo_v)

        def c_g(c):
            return cw(2 + 3 * c, wg_hbm.at[:, pl.ds(pl.multiple_of(c * FC, FC), FC)], wg_v.at[c])

        def c_u(c):
            return cw(3 + 3 * c, wu_hbm.at[:, pl.ds(pl.multiple_of(c * FC, FC), FC)], wu_v.at[c])

        def c_d(c):
            return cw(4 + 3 * c, wdT_hbm.at[:, pl.ds(pl.multiple_of(c * FC, FC), FC)], wd_v.at[c])

        def c_x(b):
            return pltpu.make_async_copy(x_hbm.at[:, pl.ds(pl.multiple_of(b * TM, TM), TM)], xin.at[b], xsem.at[b])

        def c_o(b):
            return pltpu.make_async_copy(ost.at[b], out_hbm.at[:, pl.ds(pl.multiple_of(b * TM, TM), TM)], osem.at[b])

        def stage_out(n):
            bF = n & (NB - 1)
            ost[bF] = xout[bF].astype(BF16)

        def finish_f(n):
            bF = n & (NB - 1)
            ost[bF] = xout[bF].astype(BF16)

            @pl.when(n >= NB)
            def _():
                c_o(bF).start()

        def start_group(g):
            for i in range(FU):
                c = g * FU + i
                c_g(c).start()
                c_u(c).start()
                c_d(c).start()

        with sc('prologue'):
            c_x(0).start()
            for c in range(3):
                c_qkv(c).start()
            if LATE is None:
                c_wo().start()
                for b in range(1, LA):
                    c_x(b).start()

            def zbody(i, carry):
                kext[i // NP, i % NP] = jnp.zeros(kext.shape[2:], F32)
                vext[i // NP, i % NP] = jnp.zeros(vext.shape[2:], F32)
                return carry
            lax.fori_loop(0, 2 * NP, zbody, 0)

            def zbody2(i, carry):
                xout[i] = jnp.zeros(xout.shape[1:], F32)
                return carry
            lax.fori_loop(0, NB, zbody2, 0)
            wqT[pl.ds(1728, 64), :] = jnp.zeros((64, D), BF16)
            wop[pl.ds(D, DP - D), :] = jnp.zeros((DP - D, D), BF16)
            for c, (start, off) in enumerate(((0, 0), (512, 64), (1152, 0))):
                c_qkv(c).wait()
                if c == LATE:
                    c_wo().start()
                    for b in range(1, LA):
                        c_x(b).start()
                if c == GSTART:
                    start_group(0)
                width = min(DP, 3 * D - start)
                wt32 = pltpu.bitcast(wqkv_v[:, pl.ds(start, width)].T, U32)
                for j in range(NP):
                    lw = min(128, D - j * 128)
                    planes[j, pl.ds(0, width // 2), pl.ds(0, lw)] = wt32[:, j * 128:j * 128 + lw]

                def st(j, dd, val, c=c):
                    lw = min(128, D - j * 128)
                    r0 = c * 512 + 32 * dd if dd < 16 else 1536 + 64 * c + 32 * (dd - 16)
                    wqT[pl.ds(r0, 32), pl.ds(j * 128, lw)] = val[:, :lw]
                _gather_rows(planes, off // 2, st)
            c_wo().wait()
            wo32 = pltpu.bitcast(wo_v[...], U32)
            for j in range(NP):
                lw = min(128, D - j * 128)
                planes[j, pl.ds(0, D // 2), pl.ds(0, lw)] = wo32[:, j * 128:j * 128 + lw]

            def st2(j, dd, val):
                lw = min(128, D - j * 128)
                wop[pl.ds(dd * 32, 32), pl.ds(j * 128, lw)] = val[:, :lw]
            _gather_rows(planes, 0, st2)
            wopT[...] = wop[...].T

        with sc('aonly'):
            def abody(m, carry):
                @pl.when(m == LA - 1)
                def _():
                    start_group(1)
                c_x(m).wait()
                t = a_tasks(m, chainA)
                t.pop('_links')
                for nm in (aplan or (['ln', 'q', 'k', 'r', 'v'] + ['c%d' % i for i in range(len(GROUPS))] + ['wo', 'ln2'])):
                    t.pop(nm)()
                assert not t
                return carry
            if apair is not None:
                assert LA == 2
                start_group(1)
                c_x(0).wait()
                c_x(1).wait()
                ts = [a_tasks(0, chainA), a_tasks(1, chainA)]
                for nm in apair:
                    ts[int(nm[0])].pop(nm[1:])()
                assert all(list(t.keys()) == ['_links'] for t in ts), ts
            elif only is None or only == 'a':
                lax.fori_loop(0, LA, abody, 0)
            for g in range(2, NC // FU):
                start_group(g)
            for b in range(LA, NB):
                c_x(b).start()

        def body(n, carry):
            @pl.when(n + LA - 1 < NB)
            def _():
                c_x(n + LA - 1).wait()
            with sc('main'):
                t = f_tasks(n)
                t.update(a_tasks(n + LA - 1, chain))
                t.pop('_links')
                for nm in plan:
                    t.pop(nm)()
                assert not t

            @pl.when(n >= NB)
            def _():
                c_o(n & (NB - 1)).start()
            return carry

        def fbody(n, carry):
            bF = n & (NB - 1)
            sF = n & (NSL - 1)
            facc[...] = jnp.zeros(facc.shape, F32)

            def cbody(cc, carry2):
                @pl.when(n == 0)
                def _():
                    for i in range(FU):
                        c = cc * FU + i
                        c_g(c).wait()
                        c_u(c).wait()
                        c_d(c).wait()
                xv = xnF[sF]
                hs = []
                for i in range(FU):
                    c = cc * FU + i
                    g = jnp.dot(xv, wg_v[c], preferred_element_type=F32)
                    u = jnp.dot(xv, wu_v[c], preferred_element_type=F32)
                    hs.append(_gelu_mul(g, u).astype(BF16))
                    if i > 0:
                        facc[...] += lax.dot_general(wd_v[c - 1], hs[i - 1], NT, preferred_element_type=F32)
                facc[...] += lax.dot_general(wd_v[cc * FU + FU - 1], hs[FU - 1], NT, preferred_element_type=F32)
                return carry2
            lax.fori_loop(0, NC // FU, cbody, 0)
            xout[bF] = xmid[bF] + 0.5 * facc[...]
            finish_f(n)
            return carry

        def segment(sg, carry):
            with sc('fonly'):
              if only is None or only == 'f':
                lax.fori_loop(jnp.where(sg == 0, 0, 2 * NB - LA + 1), jnp.where(sg == 0, 1, 2 * NB), fbody, 0)
            if only is None or only == 'm':
                lax.fori_loop(1, jnp.where(sg == 0, 2 * NB - LA + 1, 1), body, 0)
            return carry
        lax.fori_loop(0, 2, segment, 0)
        for b in range(NB):
            c_o(b).wait()

    def fn(A_x, A_wqkv, A_wo, B_x, B_w_gate, B_w_up, B_w_down):
        xT = A_x.reshape(S, D).T
        wdT = B_w_down.T
        hbm = pl.BlockSpec(memory_space=pltpu.MemorySpace.HBM)
        out = pl.pallas_call(
            kernel,
            in_specs=[hbm] * 6,
            out_specs=hbm,
            out_shape=jax.ShapeDtypeStruct((D, S), BF16),
            scratch_shapes=[
                pltpu.VMEM((NB, D, TM), BF16),
                pltpu.VMEM((NB, D, TM), BF16),
                pltpu.VMEM((D, 3 * D), BF16),
                pltpu.VMEM((D, D), BF16),
                pltpu.VMEM((NP, 320, 128), U32),
                pltpu.VMEM((DP, D), BF16),
                pltpu.VMEM((1792, D), BF16),
                pltpu.VMEM((D, DP), BF16),
                pltpu.VMEM((NC, D, FC), BF16),
                pltpu.VMEM((NC, D, FC), BF16),
                pltpu.VMEM((NC, D, FC), BF16),
                pltpu.VMEM((NB, D, TM), F32),
                pltpu.VMEM((NB, D, TM), F32),
                pltpu.VMEM((2, D, TM), F32),
                pltpu.VMEM((D, TM), F32),
                pltpu.VMEM((TM, D), BF16),
                pltpu.VMEM((NSL, TM, D), BF16),
                pltpu.VMEM((2, NP, TM, 128), F32),
                pltpu.VMEM((2, NP, 2 * XR + 8, 128), F32),
                pltpu.VMEM((2, NP, 2 * XR + 8, 128), F32),
                pltpu.VMEM((TM, DP), BF16),
                pltpu.SemaphoreType.DMA((5 + 3 * NC,)),
                pltpu.SemaphoreType.DMA((NB,)),
                pltpu.SemaphoreType.DMA((NB,)),
            ],
            compiler_params=pltpu.CompilerParams(vmem_limit_bytes=100 * 1024 * 1024),
        )(xT, A_wqkv, A_wo, B_w_gate, B_w_up, wdT)
        return out.T.reshape(1, S, D)
    return fn


def plan_default(NC=9, NS=16, tail=3):
    p = ['g0', 'ln', 'g1', 'q', 'd0', 'k', 'g2', 'r', 'v', 'd1']
    rest = []
    for c in range(3, NC):
        rest += ['g%d' % c, 'd%d' % (c - 1)]
    rest += ['d%d' % (NC - 1)]
    a = ['c%d' % s for s in range(NS)]
    nslots = len(rest) - tail
    out = []
    ai = 0
    for i, t in enumerate(rest[:nslots]):
        out.append(t)
        while ai < len(a) and (ai + 1) * nslots <= (i + 1) * len(a):
            out.append(a[ai]); ai += 1
    out += a[ai:]
    out += ['wo', rest[nslots], 'ln2'] + rest[nslots + 1:]
    return p + out


def mkplan(pos, NC=9):
    F = ['g0']
    for c in range(1, NC):
        F += ['g%d' % c, 'd%d' % (c - 1)]
    F += ['d%d' % (NC - 1)]
    order = ['ln', 'q', 'k', 'r', 'v'] + ['c%d' % i for i in range(16)] + ['wo', 'ln2']
    out = []
    for i in range(len(F) + 1):
        for a in order:
            if pos[a] == i:
                out.append(a)
        if i < len(F):
            out.append(F[i])
    return out


def P(ln=1, q=2, k=3, r=4, v=4, c0=5, c1=14, wo=15, ln2=16):
    pos = dict(ln=ln, q=q, k=k, r=r, v=v, wo=wo, ln2=ln2)
    for i in range(16):
        pos['c%d' % i] = c0 + ((c1 - c0 + 1) * i) // 16
    return mkplan(pos)


def ins(plan, task, before):
    p = list(plan)
    p.insert(p.index(before), task)
    return p


def AP(kind=0):
    Pn = ['ln', 'q', 'k', 'r', 'v']
    C = ['c%d' % i for i in range(16)]
    if kind == 0:
        return ['0' + t for t in Pn] + ['1' + t for t in Pn] + ['0' + t for t in C + ['wo', 'ln2']] + ['1' + t for t in C + ['wo', 'ln2']]
    if kind == 1:
        return ['0' + t for t in Pn] + ['1ln'] + ['0' + t for t in C] + ['1q', '1k', '1r', '1v'] + ['0wo', '0ln2'] + ['1' + t for t in C + ['wo', 'ln2']]


def AP2(s):
    out = []
    for t in s.split():
        if t[0] == 'C':
            idx = range(16) if len(t) == 2 else (range(8) if t[2] == 'a' else range(8, 16))
            out += [t[1] + 'c%d' % i for i in idx]
        else:
            out.append(t)
    return out


_impl = make(512, P(0, 2, 3, 3, 4, 4, 14, 15, 16), LA=2, chain=2, chainA=2, apair=AP(0))


@jax.jit
def pallas_interleave_layers__sliding_local_dilated__glu_gated_geglu__prompt_kernel(
    A_x, A_wqkv, A_wo, B_x, B_w_gate, B_w_up, B_w_down):
    return _impl(A_x, A_wqkv, A_wo, B_x, B_w_gate, B_w_up, B_w_down)
```

```python
import functools

import jax
import jax.numpy as jnp
from jax import lax
import jax.experimental.pallas as pl
import jax.experimental.pallas.tpu as pltpu

S, D, DF, H, DH, W, DIL = 2048, 576, 4608, 32, 18, 8, 2
DP = 640
NP = 5
TM = 256
NB = S // TM
SB = 128
XH = 112
XR = XH + SB
FC = 512
NC = DF // FC
FU = 3
NSL = 4
CHAIN = 2
LOG2E = 1.4426950408889634
QSCALE = float(DH ** -0.5) * LOG2E
NEG = -1e9 * LOG2E
F32, BF16, U32 = jnp.float32, jnp.bfloat16, jnp.uint32
NT = (((1,), (1,)), ((), ()))
GROUPS = [(sb, j) for sb in range(TM // SB) for j in range(8)]

STEP_PLAN = ['ln', 'g0', 'g1', 'q', 'd0', 'k', 'r', 'g2', 'v', 'c0', 'c1', 'd1', 'c2', 'g3', 'c3', 'c4',
             'd2', 'c5', 'g4', 'c6', 'c7', 'd3', 'c8', 'g5', 'c9', 'c10', 'd4', 'c11', 'g6', 'c12', 'c13',
             'd5', 'c14', 'g7', 'c15', 'd6', 'wo', 'g8', 'ln2', 'd7', 'd8']
_PRE = ['ln', 'q', 'k', 'r', 'v']
_POST = ['c%d' % i for i in range(len(GROUPS))] + ['wo', 'ln2']
PAIR_PLAN = [(0, t) for t in _PRE] + [(1, t) for t in _PRE] + [(0, t) for t in _POST] + [(1, t) for t in _POST]


def _ln_t(x):
    m = jnp.mean(x, axis=0, keepdims=True)
    xc = x - m
    v = jnp.mean(xc * xc, axis=0, keepdims=True)
    return xc * lax.rsqrt(v + 1e-5)


def _gelu2_mul(g, u):
    c0 = 0.7978845608028654
    c1 = 0.7978845608028654 * 0.044715
    t = jnp.tanh(g * (c0 + c1 * (g * g)))
    return (g * u) * (t + 1.0)


def _perm_tokens(x):
    lane = lax.broadcasted_iota(jnp.int32, (x.shape[0], 128), 1)
    idx = 16 * ((lane >> 1) & 7) + 2 * (lane >> 4) + (lane & 1)
    parts = [jnp.take_along_axis(x[:, t * 128:(t + 1) * 128], idx, axis=1) for t in range(TM // 128)]
    return jnp.concatenate(parts, axis=1)


def _gather_rows(planes, off2, store):
    for j in range(NP):
        for d2 in range(DH // 2):
            a = planes[j, pl.ds(off2 + d2, 16, stride=DH), :]
            b = planes[j, pl.ds(off2 + d2 + DH // 2, 16, stride=DH), :]
            ev = (a & jnp.uint32(0xFFFF)) | (b << 16)
            od = (a >> 16) | (b & jnp.uint32(0xFFFF0000))
            store(j, 2 * d2, pltpu.bitcast(ev, BF16))
            store(j, 2 * d2 + 1, pltpu.bitcast(od, BF16))


def _kernel(x_hbm, wqkv_hbm, wo_hbm, wg_hbm, wu_hbm, wdt_hbm, out_hbm,
            xin, ost, wqkv_v, wo_v, planes, wop, wqt, wopt, wg_v, wu_v, wd_v,
            xmid, xout, xa, facc, xna, xnf, qbuf, kext, vext, obuf, wsem, xsem, osem):

    def a_ln(m):
        b = m & (NB - 1)
        x = jnp.where(m < NB, xin[b].astype(F32), xout[b])
        xa[m & 1] = x
        xn = pltpu.bitcast(_ln_t(x).astype(BF16), U32)
        xna[...] = pltpu.bitcast(_perm_tokens(xn), BF16).T

    def mm(r0, nt):
        return lax.dot_general(xna[...], wqt[pl.ds(r0, nt * 128), :], NT, preferred_element_type=F32)

    def put_ext(m, ext, j, val):
        b = m & (NB - 1)
        cur = m & 1
        prv = 1 - cur
        for sb in range(TM // SB):
            ext[cur, j, pl.ds(sb * XR + XH, SB), :] = val[sb * SB:(sb + 1) * SB, :]
        rep = jnp.broadcast_to(val[0:1, :], (8, 128))
        top2 = lax.broadcasted_iota(jnp.int32, (8, 128), 0) < 2
        for dl in range(1, 8):
            ph = ext[prv, j, pl.ds((TM // SB - 1) * XR + XH + 16 * dl + 8, 8), :]
            ph = pltpu.roll(jnp.where(b == 0, rep, ph), 2, 0)
            for sb in range(TM // SB):
                r0 = sb * SB + 16 * dl
                lo = pltpu.roll(val[r0:r0 + 8, :], 2, 0)
                hi = pltpu.roll(val[r0 + 8:r0 + 16, :], 2, 0)
                ext[cur, j, pl.ds(sb * XR + 16 * (dl - 1), 8), :] = jnp.where(top2, ph, lo)
                ext[cur, j, pl.ds(sb * XR + 16 * (dl - 1) + 8, 8), :] = jnp.where(top2, lo, hi)
                ph = hi

    def a_q(m):
        qv = mm(0, 4)
        for j in range(4):
            qbuf[m & 1, j] = qv[:, j * 128:(j + 1) * 128] * QSCALE

    def a_kv(m, c, ext):
        kv = mm(512 * c, 4)
        for j in range(4):
            put_ext(m, ext, j, kv[:, j * 128:(j + 1) * 128])

    def a_rem(m):
        rv = mm(1536, 2)
        ta = rv[:, 0:128]
        lane = lax.broadcasted_iota(jnp.int32, (TM, 128), 1)
        qbuf[m & 1, 4] = jnp.where(lane < 64, ta * QSCALE, 0.0)
        put_ext(m, kext, 4, pltpu.roll(ta, 64, 1))
        put_ext(m, vext, 4, rv[:, 128:256])

    def a_core(m, sb, jg, links):
        b = m & (NB - 1)
        cur = m & 1
        r = sb * SB + 16 * jg
        q = [qbuf[cur, j, pl.ds(r, 16), :] for j in range(NP)]
        if len(links) >= CHAIN:
            z = links.pop(0)
            q = [pltpu.bitcast(pltpu.bitcast(x, U32) | z, F32) for x in q]
        lg = []
        for w in range(W):
            o = sb * XR + 16 * (jg - w + 7)
            acc = q[0] * kext[cur, 0, pl.ds(o, 16), :]
            for j in range(1, NP):
                acc = acc + q[j] * kext[cur, j, pl.ds(o, 16), :]
            acc = acc + pltpu.roll(acc, 64, 1)
            acc = acc + pltpu.roll(acc, 32, 1)
            if sb == 0 and w > jg:
                row = lax.broadcasted_iota(jnp.int32, (16, 128), 0)
                acc = jnp.where(jnp.logical_and(row < 2, b == 0), NEG, acc)
            lg.append(acc)
        mx = lg[0]
        for w in range(1, W):
            mx = jnp.maximum(mx, lg[w])
        e = [jnp.exp2(x - mx) for x in lg]
        s = e[0]
        for w in range(1, W):
            s = s + e[w]
        inv = 1.0 / s
        links.append(pltpu.bitcast(inv, U32) >> 31)
        for j in range(NP):
            acc = e[0] * vext[cur, j, pl.ds(sb * XR + 16 * (jg + 7), 16), :]
            for w in range(1, W):
                acc = acc + e[w] * vext[cur, j, pl.ds(sb * XR + 16 * (jg - w + 7), 16), :]
            obuf[pl.ds(r, 16), j * 128:(j + 1) * 128] = (acc * inv).astype(BF16)

    def a_wo(m):
        x1 = xa[m & 1] + _perm_tokens(lax.dot_general(wopt[...], obuf[...], NT, preferred_element_type=F32))
        xa[m & 1] = x1
        xmid[m & (NB - 1)] = x1

    def a_ln2(m):
        xnf[m & (NSL - 1)] = _ln_t(xa[m & 1]).astype(BF16).T

    def a_tasks(m):
        tasks = {
            'ln': lambda: a_ln(m),
            'q': lambda: a_q(m),
            'k': lambda: a_kv(m, 1, kext),
            'v': lambda: a_kv(m, 2, vext),
            'r': lambda: a_rem(m),
            'wo': lambda: a_wo(m),
            'ln2': lambda: a_ln2(m),
        }
        links = []
        for i, (sb, jg) in enumerate(GROUPS):
            tasks['c%d' % i] = functools.partial(a_core, m, sb, jg, links)
        return tasks

    def f_act(xv, c):
        g = jnp.dot(xv, wg_v[c], preferred_element_type=F32)
        u = jnp.dot(xv, wu_v[c], preferred_element_type=F32)
        return _gelu2_mul(g, u).astype(BF16)

    def f_down(c, h):
        return lax.dot_general(wd_v[c], h, NT, preferred_element_type=F32)

    def f_tasks(n):
        bf = n & (NB - 1)
        hvals = {}

        def f_gu(c):
            hvals[c] = f_act(xnf[n & (NSL - 1)], c)

        def f_d(c):
            y = f_down(c, hvals.pop(c))
            if c > 0:
                y = facc[...] + y
            if c == NC - 1:
                y = xmid[bf] + 0.5 * y
                xout[bf] = y
                ost[bf] = y.astype(BF16)
            else:
                facc[...] = y

        tasks = {}
        for c in range(NC):
            tasks['g%d' % c] = functools.partial(f_gu, c)
            tasks['d%d' % c] = functools.partial(f_d, c)
        return tasks

    def cw(i, src, dst):
        return pltpu.make_async_copy(src, dst, wsem.at[i])

    def c_qkv(c):
        lo, hi = ((0, 640), (640, 1152), (1152, 1728))[c]
        return cw(1 + 3 * NC + c, wqkv_hbm.at[:, pl.ds(lo, hi - lo)], wqkv_v.at[:, pl.ds(lo, hi - lo)])

    def c_wo():
        return cw(0, wo_hbm, wo_v)

    def c_ffn(c):
        col = pl.ds(pl.multiple_of(c * FC, FC), FC)
        return [cw(1 + 3 * c, wg_hbm.at[:, col], wg_v.at[c]),
                cw(2 + 3 * c, wu_hbm.at[:, col], wu_v.at[c]),
                cw(3 + 3 * c, wdt_hbm.at[:, col], wd_v.at[c])]

    def c_x(b):
        return pltpu.make_async_copy(x_hbm.at[:, pl.ds(pl.multiple_of(b * TM, TM), TM)], xin.at[b], xsem.at[b])

    def c_o(b):
        return pltpu.make_async_copy(ost.at[b], out_hbm.at[:, pl.ds(pl.multiple_of(b * TM, TM), TM)], osem.at[b])

    def start_group(g):
        for i in range(FU):
            for cp in c_ffn(g * FU + i):
                cp.start()

    c_x(0).start()
    for c in range(3):
        c_qkv(c).start()
    c_wo().start()
    c_x(1).start()

    def zero_ext(i, carry):
        kext[i // NP, i % NP] = jnp.zeros(kext.shape[2:], F32)
        vext[i // NP, i % NP] = jnp.zeros(vext.shape[2:], F32)
        return carry
    lax.fori_loop(0, 2 * NP, zero_ext, 0)

    def zero_xout(i, carry):
        xout[i] = jnp.zeros(xout.shape[1:], F32)
        return carry
    lax.fori_loop(0, NB, zero_xout, 0)
    wqt[pl.ds(1728, 64), :] = jnp.zeros((64, D), BF16)
    wop[pl.ds(D, DP - D), :] = jnp.zeros((DP - D, D), BF16)

    for c, (start, off) in enumerate(((0, 0), (512, 64), (1152, 0))):
        c_qkv(c).wait()
        if c == 2:
            start_group(0)
        width = min(DP, 3 * D - start)
        wt32 = pltpu.bitcast(wqkv_v[:, pl.ds(start, width)].T, U32)
        for j in range(NP):
            lw = min(128, D - j * 128)
            planes[j, pl.ds(0, width // 2), pl.ds(0, lw)] = wt32[:, j * 128:j * 128 + lw]

        def st_qkv(j, dd, val, c=c):
            lw = min(128, D - j * 128)
            r0 = c * 512 + 32 * dd if dd < 16 else 1536 + 64 * c + 32 * (dd - 16)
            wqt[pl.ds(r0, 32), pl.ds(j * 128, lw)] = val[:, :lw]
        _gather_rows(planes, off // 2, st_qkv)

    c_wo().wait()
    wo32 = pltpu.bitcast(wo_v[...], U32)
    for j in range(NP):
        lw = min(128, D - j * 128)
        planes[j, pl.ds(0, D // 2), pl.ds(0, lw)] = wo32[:, j * 128:j * 128 + lw]

    def st_wo(j, dd, val):
        lw = min(128, D - j * 128)
        wop[pl.ds(dd * 32, 32), pl.ds(j * 128, lw)] = val[:, :lw]
    _gather_rows(planes, 0, st_wo)
    wopt[...] = wop[...].T

    start_group(1)
    c_x(0).wait()
    c_x(1).wait()
    pair = [a_tasks(0), a_tasks(1)]
    for i, name in PAIR_PLAN:
        pair[i][name]()
    for g in range(2, NC // FU):
        start_group(g)
    for b in range(2, NB):
        c_x(b).start()

    def step(n, carry):
        @pl.when(n + 1 < NB)
        def _():
            c_x(n + 1).wait()

        tasks = f_tasks(n)
        tasks.update(a_tasks(n + 1))
        for name in STEP_PLAN:
            tasks[name]()

        @pl.when(n >= NB)
        def _():
            c_o(n & (NB - 1)).start()
        return carry

    def ffn_only(n, carry):
        bf = n & (NB - 1)
        facc[...] = jnp.zeros(facc.shape, F32)

        def chunks(cc, carry2):
            @pl.when(n == 0)
            def _():
                for i in range(FU):
                    for cp in c_ffn(cc * FU + i):
                        cp.wait()

            xv = xnf[n & (NSL - 1)]
            hs = []
            for i in range(FU):
                hs.append(f_act(xv, cc * FU + i))
                if i > 0:
                    facc[...] += f_down(cc * FU + i - 1, hs[i - 1])
            facc[...] += f_down(cc * FU + FU - 1, hs[FU - 1])
            return carry2
        lax.fori_loop(0, NC // FU, chunks, 0)
        y = xmid[bf] + 0.5 * facc[...]
        xout[bf] = y
        ost[bf] = y.astype(BF16)

        @pl.when(n >= NB)
        def _():
            c_o(bf).start()
        return carry

    def segment(sg, carry):
        lax.fori_loop(jnp.where(sg == 0, 0, 2 * NB - 1), jnp.where(sg == 0, 1, 2 * NB), ffn_only, 0)
        lax.fori_loop(1, jnp.where(sg == 0, 2 * NB - 1, 1), step, 0)
        return carry
    lax.fori_loop(0, 2, segment, 0)

    for b in range(NB):
        c_o(b).wait()


@jax.jit
def pallas_interleave_layers__sliding_local_dilated__glu_gated_geglu__prompt_kernel(
    A_x: jax.Array,
    A_wqkv: jax.Array,
    A_wo: jax.Array,
    B_x: jax.Array,
    B_w_gate: jax.Array,
    B_w_up: jax.Array,
    B_w_down: jax.Array,
):
    hbm = pl.BlockSpec(memory_space=pltpu.MemorySpace.HBM)
    out = pl.pallas_call(
        _kernel,
        in_specs=[hbm] * 6,
        out_specs=hbm,
        out_shape=jax.ShapeDtypeStruct((D, S), BF16),
        scratch_shapes=[
            pltpu.VMEM((NB, D, TM), BF16),
            pltpu.VMEM((NB, D, TM), BF16),
            pltpu.VMEM((D, 3 * D), BF16),
            pltpu.VMEM((D, D), BF16),
            pltpu.VMEM((NP, DP // 2, 128), U32),
            pltpu.VMEM((DP, D), BF16),
            pltpu.VMEM((14 * 128, D), BF16),
            pltpu.VMEM((D, DP), BF16),
            pltpu.VMEM((NC, D, FC), BF16),
            pltpu.VMEM((NC, D, FC), BF16),
            pltpu.VMEM((NC, D, FC), BF16),
            pltpu.VMEM((NB, D, TM), F32),
            pltpu.VMEM((NB, D, TM), F32),
            pltpu.VMEM((2, D, TM), F32),
            pltpu.VMEM((D, TM), F32),
            pltpu.VMEM((TM, D), BF16),
            pltpu.VMEM((NSL, TM, D), BF16),
            pltpu.VMEM((2, NP, TM, 128), F32),
            pltpu.VMEM((2, NP, 2 * XR + 8, 128), F32),
            pltpu.VMEM((2, NP, 2 * XR + 8, 128), F32),
            pltpu.VMEM((TM, DP), BF16),
            pltpu.SemaphoreType.DMA((4 + 3 * NC,)),
            pltpu.SemaphoreType.DMA((NB,)),
            pltpu.SemaphoreType.DMA((NB,)),
        ],
        compiler_params=pltpu.CompilerParams(vmem_limit_bytes=100 * 1024 * 1024),
    )(A_x.reshape(S, D).T, A_wqkv, A_wo, B_w_gate, B_w_up, B_w_down.T)
    return out.T.reshape(1, S, D)
```
